```python
import os as _os
_os.environ.setdefault("JAX_PLATFORMS", "cpu")
import jax
import jax.numpy as jnp

def _softmax(x, axis=-1):
    return jax.nn.softmax(x, axis=axis)
def _gelu(x):
    return jax.nn.gelu(x, approximate=True)
def _silu(x):
    return jax.nn.silu(x)
def _sigmoid(x):
    return jax.nn.sigmoid(x)
def _layernorm(x, axis=-1, eps=1e-5):
    m = jnp.mean(x, axis=axis, keepdims=True)
    v = jnp.var(x, axis=axis, keepdims=True)
    return (x - m) / jnp.sqrt(v + eps)
def _scatter_add(tgt, idx, src, axis=0):
    return tgt.at[idx].add(src)
def _segment_sum(src, seg, n):
    return jax.ops.segment_sum(src, seg, n)
class _Rng:
    def __init__(self, key):
        self._k = key
    def _next(self):
        self._k, sub = jax.random.split(self._k)
        return sub
    def normal(self, shape):
        return jax.random.normal(self._next(), shape, dtype=jnp.bfloat16)
    def randint(self, lo, hi, shape):
        return jax.random.randint(self._next(), shape, lo, hi, dtype=jnp.int32)
    def uniform(self, shape, lo=0.0, hi=1.0):
        return jax.random.uniform(self._next(), shape, jnp.bfloat16, lo, hi)
    def permutation(self, n):
        return jax.random.permutation(self._next(), n)


kernel_name = 'concat_heads__mha_block__spectral_gfnet__prompt'

def setup_inputs():
    _rng = _Rng(jax.random.key(int.from_bytes(__import__("os").urandom(4), "little")))
    _w = (lambda a: (lambda t: t.astype(jnp.bfloat16) if jnp.issubdtype(t.dtype, jnp.floating) else t)(jnp.asarray(a)))
    def _A_setup():
        B, S, D, H = 1, 2048, 512, 32
        return {
            "x": _w((lambda *s: _rng.normal(s) * 0.2)(B, S, D)),
            "wqkv": _w((lambda *s: _rng.normal(s) * 0.2)(D, 3 * D)),
            "wo": _w((lambda *s: _rng.normal(s) * 0.05)(D, D)),
        }
    _A_in = _A_setup()

    def _B_setup():
        B, S, D = 1, 2048, 512
        Df = D // 2 + 1
        return {
            "x": _w((lambda *s: _rng.normal(s) * 0.05)(B, S, D)),
            "w_r": _w((lambda *s: _rng.normal(s) * 0.05)(S, Df) * 0.02),
            "w_i": _w((lambda *s: _rng.normal(s) * 0.05)(S, Df) * 0.02),
        }
    _B_in = _B_setup()

    return {
        "A_x": _A_in["x"],
        "A_wqkv": _A_in["wqkv"],
        "A_wo": _A_in["wo"],
        "B_x": _B_in["x"],
        "B_w_r": _B_in["w_r"],
        "B_w_i": _B_in["w_i"],
    }

def reference(A_x, A_wqkv, A_wo, B_x, B_w_r, B_w_i):
    def _A_ref(x, wqkv, wo):
        B, S, D = x.shape
        H = 32
        Dh = D // H
        qkv = (lambda x, *d: x.transpose(*d))((x @ wqkv).reshape(B, S, 3, H, Dh), 2, 0, 3, 1, 4)
        q, k, v = qkv[0], qkv[1], qkv[2]
        scores = jnp.einsum("bhqd,bhkd->bhqk", q, k) * (Dh ** -0.5)
        p = _softmax(scores, axis=-1)
        o = jnp.einsum("bhqk,bhkd->bhqd", p, v)
        return (lambda x, *d: x.transpose(*d))(o, 0, 2, 1, 3).reshape(B, S, D) @ wo

    def _B_ref(x, w_r, w_i):
        B, S, D = x.shape
        X = (lambda x, axes=(-2,-1): jnp.fft.rfft2(x.astype(jnp.float32), axes=axes))(x, axes=(-2, -1))
        W = w_r + 1j * w_i
        X = X * W
        y = (lambda x, s, axes=(-2,-1): jnp.fft.irfft2(x, s=s, axes=axes).astype(jnp.bfloat16))(X, (S, D), axes=(-2, -1))
        return y

    a = _A_ref(A_x, A_wqkv, A_wo)
    b = _B_ref(B_x, B_w_r, B_w_i)
    return jnp.concatenate([a, b], axis=-1)
```

```python
import functools
import math

import jax
import jax.numpy as jnp
import numpy as np
from jax import lax
import jax.experimental.pallas as pl
import jax.experimental.pallas.tpu as pltpu

S, D, H, DH = 2048, 512, 32, 16
F32, BF16, U32 = jnp.float32, jnp.bfloat16, jnp.uint32

CFG = dict(g=40, phase=128, shift=9, nz=64, prep_at=(16, 48), proj_rows=256, out_rows=256, f1_rows=16,
           heads_per_iter=2, only=None)


def _dft_constants():
    n = np.arange(256)[:, None]
    m = np.arange(128)[None, :]
    inv = 1.0 / (S * D)
    sign = (-1.0) ** np.arange(256)
    mats = []
    for odd in (0, 1):
        ang = 2.0 * np.pi * ((n * (2 * m + odd)) % D) / D
        fwd = np.concatenate([np.cos(ang), -np.sin(ang)], axis=1)
        bwd = 2.0 * inv * fwd.T.copy()
        if not odd:
            fwd[:, 128] = sign
            bwd[0] = inv
            bwd[128] = inv * sign
        mats += [fwd, bwd]
    dmat = np.stack([mats[0], mats[2], mats[1], mats[3]])

    b = np.arange(64)[None, None, :]
    f = np.arange(32)[:, None, None] + 32 * np.arange(64)[None, :, None]
    ang = 2.0 * np.pi * ((b * f) % S) / S
    c, s = np.cos(ang), -np.sin(ang)
    g = np.concatenate([np.concatenate([c, -s], axis=2), np.concatenate([s, c], axis=2)], axis=1)
    gmat = np.concatenate([g, g.transpose(0, 2, 1)], axis=0)

    e = np.arange(128)
    a = np.arange(16)
    ang = 2.0 * np.pi * ((e[:, None] * a[None, :]) % 16) / 16
    c, s = np.cos(ang), -np.sin(ang)
    n1 = np.zeros((256, 128))
    n1[:128, :16], n1[128:, :16] = c, s
    n1[:128, 32:48], n1[:128, 48:64] = c, s
    n1[128:, 32:48], n1[128:, 48:64] = -s, c
    n2 = np.zeros((48, 256))
    n2[:16, :128], n2[:16, 128:] = c.T, -s.T
    n2[16:32, :128], n2[16:32, 128:] = s.T, c.T
    n2[32:, :128], n2[32:, 128:] = c.T, s.T
    ang = 2.0 * np.pi * (e[:, None] * e[None, :]) / S
    tw = np.concatenate([np.cos(ang), -np.sin(ang)], axis=0)
    nyq = np.concatenate([n1, tw, n2[:, :128], n2[:, 128:]], axis=0)
    return dmat.astype(jnp.bfloat16), gmat.astype(jnp.bfloat16), nyq.astype(np.float32)


_DMAT, _GMAT, _NYQ = _dft_constants()


def _fft(x):
    n = len(x)
    if n == 1:
        return x
    if n == 2:
        (ar, ai), (br, bi) = x
        return [(ar + br, ai + bi), (ar - br, ai - bi)]
    u, z1, z3 = _fft(x[0::2]), _fft(x[1::4]), _fft(x[3::4])

    def twiddle(z, k):
        zr, zi = z
        if k == 0:
            return zr, zi
        c, s = math.cos(2 * math.pi * k / n), -math.sin(2 * math.pi * k / n)
        if 8 * k == n:
            return (zr + zi) * c, (zi - zr) * c
        if 8 * k == 3 * n:
            return (zi - zr) * -c, (zr + zi) * c
        return zr * c - zi * s, zr * s + zi * c

    out = [None] * n
    for k in range(n // 4):
        (ar, ai), (br, bi) = twiddle(z1[k], k), twiddle(z3[k], 3 * k)
        sr, si, dr, di = ar + br, ai + bi, ar - br, ai - bi
        (ur, ui), (vr, vi) = u[k], u[k + n // 4]
        out[k] = (ur + sr, ui + si)
        out[k + n // 2] = (ur - sr, ui - si)
        out[k + n // 4] = (vr + di, vi - dr)
        out[k + 3 * n // 4] = (vr - di, vi + dr)
    return out


def _ifft(x):
    return [(r, i) for i, r in _fft([(i, r) for r, i in x])]


def _fft_order(idx):
    if len(idx) <= 2:
        return list(idx)
    return _fft_order(idx[0::2]) + _fft_order(idx[1::4]) + _fft_order(idx[3::4])


def _dot(a, b):
    return lax.dot_general(a, b, (((1,), (0,)), ((), ())), preferred_element_type=F32)


def _dot_nt(a, b):
    return lax.dot_general(a, b, (((1,), (1,)), ((), ())), preferred_element_type=F32)


def _key_plan(g, phase):
    plan, cnt = [], [0, 0]
    for i in range(256):
        on_vpu = int(((i + 1) * g + phase) // 256 > (i * g + phase) // 256)
        plan.append((on_vpu, cnt[on_vpu], 16 * (i // 16) + 15 - i % 16))
        cnt[on_vpu] += 1
    return plan


def _mxu_order(plan, shift, units):
    nm = sum(1 for p in plan if not p[0]) // 2
    ops, done = [], 0
    for t in range(16 * units):
        u, kb = divmod(t, 16)
        need = u * nm + max(i for v, i, _ in plan[16 * kb:16 * kb + 16] if not v) // 2 + 1
        target = min(need + shift, units * nm)
        while done < target:
            uu = done // nm
            end = min(target, (uu + 1) * nm)
            ops.append(("qk", uu, done - uu * nm, end - uu * nm))
            done = end
        ops.append(("pv", u, kb))
    return ops


def _kernel(cfg, ax_hbm, wqkv_hbm, wo_hbm, bx_hbm, wr_hbm, wi_hbm, dmat_hbm, gmat_hbm, nyq_hbm, out_hbm,
            ax_ref, wqkv_ref, wo_ref, bx_ref, wr_ref, wi_ref, dmat_ref, gmat_ref, nyq_ref,
            qt_ref, km_ref, kv_ref, vt_ref, ot_ref, kh0_ref, kh1_ref, kb0_ref, kb1_ref,
            u_ref, v_ref, w_ref, n_ref, ya_ref, yb_ref, bad_ref, kf_ref, zero_ref, in_sem, out_sem):
    G, PR, OR = cfg["g"], cfg["proj_rows"], cfg["out_rows"]
    only = cfg["only"]
    plan = _key_plan(G, cfg["phase"])
    NX = S // PR

    def cols(ref, i):
        return ref.at[:, pl.ds(i * D, D)]

    pairs = [(ax_hbm.at[pl.ds(0, PR)], ax_ref.at[pl.ds(0, PR)])]
    pairs += [(cols(wqkv_hbm, i), cols(wqkv_ref, i)) for i in range(3)]
    pairs += [(ax_hbm.at[pl.ds(i * PR, PR)], ax_ref.at[pl.ds(i * PR, PR)]) for i in range(1, NX)]
    pairs += [(bx_hbm, bx_ref), (dmat_hbm, dmat_ref), (wr_hbm, wr_ref), (wi_hbm, wi_ref),
              (gmat_hbm, gmat_ref), (nyq_hbm, nyq_ref), (wo_hbm, wo_ref)]
    copies = [pltpu.make_async_copy(s, d, in_sem.at[i]) for i, (s, d) in enumerate(pairs)]
    for c in copies:
        c.start()
    cp_x = [copies[0]] + copies[4:3 + NX]
    cp_w = copies[1:4]
    cp_bx, cp_dmat, cp_wr, cp_wi, cp_gmat, cp_nyq, cp_wo = copies[3 + NX:]

    def fill(i, c):
        zero_ref[i] = 0
        return c

    lax.fori_loop(0, cfg["nz"], fill, 0)

    qscale = DH ** -0.5 * math.log2(math.e)
    pending = {}
    for i in range(NX):
        cp_x[i].wait()
        rows = slice(i * PR, (i + 1) * PR)
        x = ax_ref[rows, :]
        if i == 0:
            cp_w[0].wait()
        q = _dot(x, wqkv_ref[:, 0:D]) * qscale
        qt_ref[:, :, rows] = q.T.reshape(H, DH, PR)
        if i == 0:
            cp_w[1].wait()
        k = _dot(x, wqkv_ref[:, D:2 * D])
        for on_vpu, idx, grp in plan[i * PR // 8:(i + 1) * PR // 8]:
            piece = k[grp * 8 - i * PR:(grp + 1) * 8 - i * PR]
            if on_vpu:
                for j in range(4):
                    kv_ref[j, idx * 8:(idx + 1) * 8, :] = piece[:, j * 128:(j + 1) * 128]
            elif idx % 2 == 0:
                pending[idx] = piece
            else:
                both = jnp.concatenate([pending.pop(idx - 1), piece], axis=0).astype(BF16)
                both = pltpu.bitcast(both, U32)
                for j in range(4):
                    km_ref[j, (idx // 2) * 8:(idx // 2 + 1) * 8, :] = both[:, j * 128:(j + 1) * 128]
        if i == 0:
            cp_w[2].wait()
        v = _dot(x, wqkv_ref[:, 2 * D:3 * D])
        vt_ref[:, :, rows] = pltpu.bitcast(v.T.astype(BF16), U32).reshape(H, DH // 2, PR)

    R = cfg["f1_rows"]
    order = _fft_order(list(range(32)))
    lane0 = lax.broadcasted_iota(jnp.int32, (8, 128), 1) == 0
    cp_bx.wait()
    cp_dmat.wait()

    def forward(j, c):
        b0 = pl.multiple_of(j * R, R)
        x = jnp.concatenate([bx_ref[pl.ds(64 * a + b0, R), :].astype(F32) for a in order], axis=0)
        halves = (x[:, :256] + x[:, 256:], x[:, :256] - x[:, 256:])
        for odd in (0, 1):
            z = _dot(halves[odd], dmat_ref[odd])
            for r in range(R // 8):
                seq = [None] * 32
                for pos, a in enumerate(order):
                    blk = z[pos * R + r * 8:pos * R + r * 8 + 8]
                    re, im = blk[:, :128], blk[:, 128:]
                    if not odd:
                        n_ref[pl.ds(64 * a + b0 + r * 8, 8), :] = im
                        im = jnp.where(lane0, 0.0, im)
                    seq[a] = (re, im)
                for f1, (re, im) in enumerate(_fft(seq)):
                    u_ref[f1, pl.ds(b0 + r * 8, 8), odd * 128:(odd + 1) * 128] = re
                    u_ref[f1, pl.ds(64 + b0 + r * 8, 8), odd * 128:(odd + 1) * 128] = im
        return c

    lax.fori_loop(0, 64 // R, forward, 0)

    cp_wr.wait()
    cp_wi.wait()
    cp_gmat.wait()
    cp_nyq.wait()
    for i, ref in enumerate((wr_ref, wi_ref)):
        for t in range(16):
            w_ref[i, t * 128:(t + 1) * 128, :] = pltpu.bitcast(ref[0:256, t * 128:(t + 1) * 128], U32).T

    zn = jnp.concatenate([n_ref[t * 128:(t + 1) * 128, :].T[0:1] for t in range(16)], axis=0)
    wn = [jnp.concatenate([ref[256:257, t * 128:(t + 1) * 128].astype(F32) for t in range(16)], axis=0)
          for ref in (wr_ref, wi_ref)]
    twr, twi = nyq_ref[256:384, :], nyq_ref[384:512, :]
    t = _dot(nyq_ref[0:256, 0:16], zn)
    tr, ti = t[:128], t[128:]
    t = jnp.concatenate([tr * twr - ti * twi, tr * twi + ti * twr], axis=1)
    zf = _dot_nt(jnp.concatenate([nyq_ref[512:544, :], nyq_ref[560:592, :]], axis=1), t)
    zr, zi = zf[:16], zf[16:]
    yf = jnp.concatenate([zr * wn[0] - zi * wn[1], zr * wn[1] + zi * wn[0]], axis=0)
    t = _dot(nyq_ref[0:256, 32:64], yf)
    tr, ti = t[:128], t[128:]
    t = jnp.concatenate([tr * twr + ti * twi, ti * twr - tr * twi], axis=1)
    yn = _dot_nt(jnp.concatenate([nyq_ref[544:560, :], nyq_ref[592:608, :]], axis=1), t)
    for t in range(16):
        n_ref[t * 128:(t + 1) * 128, :] = jnp.broadcast_to(yn[t:t + 1], (128, 128)).T

    spec = {}
    LAG = 3
    for f1 in range(32 + LAG):
        if f1 < 32:
            t = _dot(gmat_ref[f1], u_ref[f1])
            w = []
            for i in range(2):
                bits = w_ref[i, pl.ds(f1, 64, stride=32), :]
                w.append(jnp.concatenate([pltpu.bitcast(bits << 16, F32),
                                          pltpu.bitcast(bits & np.uint32(0xFFFF0000), F32)], axis=1))
            tr, ti = t[:64], t[64:]
            spec[f1] = jnp.concatenate([tr * w[0] - ti * w[1], tr * w[1] + ti * w[0]], axis=0)
        if f1 >= LAG:
            v_ref[f1 - LAG] = _dot(gmat_ref[32 + f1 - LAG], spec.pop(f1 - LAG))

    def backward(j, c):
        b0 = pl.multiple_of(j * R, R)
        res = []
        for odd in (0, 1):
            blocks = [[None] * (R // 8) for _ in range(32)]
            for r in range(R // 8):
                seq = [(v_ref[f1, pl.ds(b0 + r * 8, 8), odd * 128:(odd + 1) * 128],
                        v_ref[f1, pl.ds(64 + b0 + r * 8, 8), odd * 128:(odd + 1) * 128]) for f1 in range(32)]
                for a, (re, im) in enumerate(_ifft(seq)):
                    if not odd:
                        im = jnp.where(lane0, n_ref[pl.ds(64 * a + b0 + r * 8, 8), :], im)
                    blocks[a][r] = jnp.concatenate([re, im], axis=1)
            res.append(_dot(jnp.concatenate([x for blk in blocks for x in blk], axis=0), dmat_ref[2 + odd]))
        y = jnp.concatenate([res[0] + res[1], res[0] - res[1]], axis=1).astype(BF16)
        for a in range(32):
            yb_ref[pl.ds(64 * a + b0, R), :] = y[a * R:(a + 1) * R]
        return c

    lax.fori_loop(0, 64 // R, backward, 0)
    cp_yb = pltpu.make_async_copy(yb_ref, out_hbm.at[:, pl.ds(D, D)], out_sem.at[0])
    cp_yb.start()

    kh, kb = (kh0_ref, kh1_ref), (kb0_ref, kb1_ref)

    def prepare(h, slot):
        grp = h // 8
        shift = (128 - DH * (h % 8)) % 128
        kh[slot][0] = pltpu.roll(km_ref[grp], shift, 1)
        kv = pltpu.roll(kv_ref[grp], shift, 1)
        for d in range(DH):
            kb[slot][0, d] = jnp.broadcast_to(kv[:, d:d + 1], (8 * G, 128))

    prepare(0, 0)
    bad_ref[...] = jnp.zeros(bad_ref.shape, F32)
    HPI = cfg["heads_per_iter"]
    ops = _mxu_order(plan, cfg["shift"], 4 * HPI)

    def heads(it, c):
        count = [0]

        def zero():
            count[0] += 1
            return zero_ref[count[0] % cfg["nz"]]

        def vpu_scores(h, slot, q0, idx):
            z = zero()
            s = None
            for d in range(DH):
                q = jnp.concatenate(
                    [jnp.broadcast_to(qt_ref[h + z, d:d + 1, q0 + j * 128:q0 + (j + 1) * 128], (8, 128))
                     for j in range(4)], axis=1)
                term = jnp.concatenate([kb[slot][z, d, idx * 8:(idx + 1) * 8, :]] * 4, axis=1) * q
                s = term if s is None else s + term
            return s

        probs, acc, den = {}, {}, {}
        for op in ops:
            u = op[1]
            slot, q0 = (u // 4) % 2, (u % 4) * 512
            h = it * HPI + u // 4
            if op[0] == "qk":
                lo, hi = op[2:]
                z = zero()
                keys = pltpu.bitcast(kh[slot][z, lo * 8:hi * 8, 0:DH], BF16)
                p = jnp.exp2(_dot(keys, qt_ref[h + z, :, q0:q0 + 512]))
                for r in range(2 * (hi - lo)):
                    probs[u, 2 * lo + r] = p[r * 8:(r + 1) * 8]
                continue
            blk = op[2]
            if (u % 4) * 16 + blk == cfg["prep_at"][0]:
                prepare(jnp.minimum(h + 1, H - 1), 1 - slot)
            tile = [jnp.exp2(vpu_scores(h, slot, q0, i)) if on_vpu else probs.pop((u, i))
                    for on_vpu, i, _ in plan[16 * blk:16 * blk + 16]]
            for p in tile:
                den[u] = den[u] + p if u in den else p
            vals = pltpu.bitcast(vt_ref[h + zero(), :, blk * 128:(blk + 1) * 128], BF16)
            o = _dot(vals, jnp.concatenate(tile[::-1], axis=0))
            acc[u] = acc[u] + o if u in acc else o
            if blk == 15:
                l = jnp.sum(den.pop(u), axis=0, keepdims=True)
                o = acc.pop(u)
                safe = (l >= 2.0 ** -20) & (l <= 2.0 ** 60) & (jnp.abs(o) <= 2.0 ** 126)
                bad_ref[...] = jnp.where(safe, bad_ref[...], 1.0)
                ot_ref[h, :, q0:q0 + 512] = pltpu.bitcast((o * (1.0 / l)).astype(BF16), U32)
        return c

    lax.fori_loop(0, H // HPI, heads, 0)

    @pl.when(jnp.max(bad_ref[...]) > 0.0)
    def _():
        def group(grp, c):
            col = pl.multiple_of(D + grp * 128, 128)

            def project(i, c):
                rows = pl.ds(pl.multiple_of(i * 256, 256), 256)
                kf_ref[rows, :] = _dot(ax_ref[rows, :], wqkv_ref[:, pl.ds(col, 128)])
                return c

            lax.fori_loop(0, S // 256, project, 0)

            def block(i, c):
                j = i // 16
                h = grp * 8 + j
                cols_q = pl.ds(pl.multiple_of((i % 16) * 128, 128), 128)
                mine = lax.broadcasted_iota(jnp.int32, (S, 128), 1) // DH == j
                keys = jnp.where(mine, kf_ref[...], 0.0)
                s = _dot(keys, jnp.concatenate([qt_ref[h, :, cols_q]] * 8, axis=0))
                p = jnp.exp2(s - jnp.max(s, axis=0, keepdims=True))
                o = _dot(pltpu.bitcast(vt_ref[h], BF16), p) / jnp.sum(p, axis=0, keepdims=True)
                ot_ref[h, :, cols_q] = pltpu.bitcast(o.astype(BF16), U32)
                return c

            return lax.fori_loop(0, 8 * 16, block, c)

        lax.fori_loop(0, 4, group, 0)

    cp_wo.wait()
    outs = []
    for i in range(S // OR):
        rows = slice(i * OR, (i + 1) * OR)
        o = pltpu.bitcast(ot_ref[:, :, rows].reshape(D // 2, OR), BF16)
        ya_ref[rows, :] = _dot(o.T, wo_ref[...]).astype(BF16)
        outs.append(pltpu.make_async_copy(ya_ref.at[pl.ds(i * OR, OR)],
                                          out_hbm.at[pl.ds(i * OR, OR), pl.ds(0, D)], out_sem.at[1 + i]))
        outs[-1].start()
    cp_yb.wait()
    for c in outs:
        c.wait()


def make(**over):
    cfg = dict(CFG, **over)
    g = cfg["g"]
    vmem = pltpu.VMEM
    scratch = [
        vmem((S, D), BF16), vmem((D, 3 * D), BF16), vmem((D, D), BF16), vmem((S, D), BF16),
        vmem((D // 2 + 1, S), BF16), vmem((D // 2 + 1, S), BF16),
        vmem(_DMAT.shape, BF16), vmem(_GMAT.shape, BF16), vmem(_NYQ.shape, F32),
        vmem((H, DH, S), F32), vmem((4, (256 - g) * 4, 128), U32), vmem((4, 8 * g, 128), F32),
        vmem((H, DH // 2, S), U32), vmem((H, DH // 2, S), U32),
        vmem((1, (256 - g) * 4, 128), U32), vmem((1, (256 - g) * 4, 128), U32),
        vmem((1, DH, 8 * g, 128), F32), vmem((1, DH, 8 * g, 128), F32),
        vmem((32, 128, 256), F32), vmem((32, 128, 256), F32), vmem((2, S, 128), U32), vmem((S, 128), F32),
        vmem((S, D), BF16), vmem((S, D), BF16), vmem((DH, 512), F32), vmem((S, 128), F32),
        pltpu.SMEM((cfg["nz"],), jnp.int32),
        pltpu.SemaphoreType.DMA((S // cfg["proj_rows"] + 10,)),
        pltpu.SemaphoreType.DMA((S // cfg["out_rows"] + 1,)),
    ]

    def fn(A_x, A_wqkv, A_wo, B_x, B_w_r, B_w_i):
        out = pl.pallas_call(
            functools.partial(_kernel, cfg),
            out_shape=jax.ShapeDtypeStruct((S, 2 * D), BF16),
            in_specs=[pl.BlockSpec(memory_space=pl.ANY)] * 9,
            out_specs=pl.BlockSpec(memory_space=pl.ANY),
            scratch_shapes=scratch,
            compiler_params=pltpu.CompilerParams(vmem_limit_bytes=100 * 1024 * 1024),
            name="mha_gfnet",
        )(A_x.reshape(S, D), A_wqkv, A_wo, B_x.reshape(S, D), B_w_r.T, B_w_i.T, _DMAT, _GMAT, _NYQ)
        return out.reshape(1, S, 2 * D)

    return jax.jit(fn)


_FN = make()


@jax.jit
def pallas_concat_heads__mha_block__spectral_gfnet__prompt_kernel(A_x, A_wqkv, A_wo, B_x, B_w_r, B_w_i):
    return _FN(A_x, A_wqkv, A_wo, B_x, B_w_r, B_w_i)
```

```python
import functools
import math

import jax
import jax.numpy as jnp
import numpy as np
from jax import lax
import jax.experimental.pallas as pl
import jax.experimental.pallas.tpu as pltpu

S, D, H, DH = 2048, 512, 32, 16
F32, BF16, U32 = jnp.float32, jnp.bfloat16, jnp.uint32

CFG = dict(g=44, phase=128, lag=152, ahead=0, form=0, nz=256, hpi=2, out_rows=(512, 512, 512, 256, 128, 128), skip=(),
           fwd_n=1, flags=None, cost=(90, 75, 145), njobs=(7, 6), split0=3, prep0=1, oput=1, slack=0.15, merge=1, slack3=0.2, slack4=0.2, spanm=19.3, lead=100, back_at=2, late=7, split=4, tgate=(4, 1), border=1, part=6, delay=0, scopes=0, chains=0, link=21, vdt='u32', gcol=4, prep_span=60,
           nyq_at=(0, 1, 2, 3), tail=1, qdt='bf16')

XP = 260
DP = 36


def _dft_constants():
    n = np.arange(128)[:, None]
    m = np.arange(64)[None, :]
    inv = 1.0 / (S * D)
    sign = (-1.0) ** np.arange(128)

    def cs(k):
        ang = 2.0 * np.pi * ((n * k) % D) / D
        return np.cos(ang), -np.sin(ang)

    (c0, s0), (c2, s2) = cs(4 * m), cs(4 * m + 2)
    f0 = np.stack([c0, s0], axis=2).reshape(128, 128)
    f2 = np.roll(np.stack([c2, s2], axis=2).reshape(128, 128), 1, axis=1)
    b0, b2 = 2.0 * inv * f0.T.copy(), 2.0 * inv * f2.T
    f0[:, 1] = sign
    b0[0], b0[1] = inv, inv * sign
    c1, s1 = cs(np.stack([4 * m + 1, D - (4 * m + 3)], axis=2).reshape(1, 128))
    dmat = np.stack([f0, f2, c1, -(c1 + s1), s1 - c1,
                     b0, b2, 2.0 * inv * c1.T, 2.0 * inv * (s1 - c1).T, -2.0 * inv * (c1 + s1).T])

    e = np.arange(128)
    a = np.arange(16)
    ang = 2.0 * np.pi * ((e[:, None] * a[None, :]) % 16) / 16
    c, s = np.cos(ang), -np.sin(ang)
    n1 = np.zeros((512, 128))
    n1[:128, :16], n1[128:256, :16] = c, s
    n1[256:384, :16], n1[256:384, 16:32] = c, s
    n1[384:, :16], n1[384:, 16:32] = -s, c
    n2 = np.zeros((48, 256))
    n2[:16, :128], n2[:16, 128:] = c.T, -s.T
    n2[16:32, :128], n2[16:32, 128:] = s.T, c.T
    n2[32:, :128], n2[32:, 128:] = c.T, s.T
    ang = 2.0 * np.pi * (e[:, None] * e[None, :]) / S
    tw = np.concatenate([np.cos(ang), -np.sin(ang)], axis=0)
    nyq = np.concatenate([n1, n2[:, :128], n2[:, 128:], np.zeros((32, 128))], axis=0)
    ang = 2.0 * np.pi * e / 128
    roots = np.zeros((1, 144, 256))
    roots[0, :128, :128], roots[0, :128, 128:] = np.cos(ang)[:, None], -np.sin(ang)[:, None]
    return dmat.astype(jnp.bfloat16), nyq.astype(jnp.bfloat16), tw.astype(np.float32), roots.astype(np.float32)


_DMAT, _NYQ, _TW, _ROOTS = _dft_constants()


def _cmul(z, c, s):
    re, im = z
    return re * c - im * s, re * s + im * c


def _pm(a, b, quarter=False):
    (ar, ai), (br, bi) = a, b
    if quarter:
        return (ar + bi, ai - br), (ar - bi, ai + br)
    return (ar + br, ai + bi), (ar - br, ai - bi)


def _dft4(x, quarter=False):
    s0, d0 = _pm(x[0], x[2], quarter)
    s1, d1 = _pm(x[1], x[3])
    (y0, y2), (y1, y3) = _pm(s0, s1), _pm(d0, d1, True)
    return [y0, y1, y2, y3]


def _dot(a, b):
    return lax.dot_general(a, b, (((1,), (0,)), ((), ())), preferred_element_type=F32)


def _dot_nt(a, b):
    return lax.dot_general(a, b, (((1,), (1,)), ((), ())), preferred_element_type=F32)


def _tile(j):
    return slice(j * 128, (j + 1) * 128)


def _key_plan(g, phase):
    plan, cnt = [], [0, 0]
    for i in range(256):
        on_vpu = int(((i + 1) * g + phase) // 256 > (i * g + phase) // 256)
        plan.append((on_vpu, cnt[on_vpu]))
        cnt[on_vpu] += 1
    return plan


def _mxu_order(plan, lag, units):
    nm = sum(1 for p in plan if not p[0]) // 2
    ops, issued, clock = [], [], 0
    for t in range(16 * units):
        u, kb = divmod(t, 16)
        pos, last = max((n, i) for n, (v, i) in enumerate(plan[16 * kb:16 * kb + 16]) if not v)
        row = u * nm + last // 2
        first = len(issued)
        while len(issued) < units * nm and (len(issued) <= row or
                                            clock < issued[row] + 8 * (last % 2) + 2 * (15 - pos) + lag):
            issued.append(clock)
            clock += 16
        while first < len(issued):
            uu = first // nm
            end = min(len(issued), (uu + 1) * nm)
            ops.append(("qk", uu, first - uu * nm, end - uu * nm))
            first = end
        ops.append(("pv", u, kb))
        clock += 16
    return ops


def _kernel(cfg, ax_hbm, wqkv_hbm, wo_hbm, bx_hbm, wr_hbm, wi_hbm, dmat_hbm, nyq_hbm, tw_hbm, roots_hbm, out_hbm,
            ax_ref, wqkv_ref, wo_ref, bx_ref, wr_ref, wi_ref, dmat_ref, nyq_ref, tw_ref, roots_ref,
            wq_ref, wv_ref, qt_ref, qm_ref, qs_ref, xk_ref, km_ref, ks_ref, vt_ref, ot_ref, den_ref, inv_ref,
            kh0_ref, kh1_ref, kb0_ref, kb1_ref, src_ref,
            fe_ref, fo_ref, twb_ref, w_ref, n_ref, ya_ref, yb_ref, kf_ref, of_ref, zero_ref, in_sem, out_sem):
    G = cfg["g"]
    skip = cfg["skip"]
    plan = _key_plan(G, cfg["phase"])
    key_order = [16 * (i // 16) + 15 - i % 16 for side in (1, 0) for i, (on_vpu, _) in enumerate(plan) if on_vpu == side]

    sems = iter(range(in_sem.shape[0]))

    def fetch(src, dst):
        return pltpu.make_async_copy(src, dst, in_sem.at[next(sems)])

    cp_x = [fetch(ax_hbm.at[pl.ds(lo, n)], ax_ref.at[0, pl.ds(lo, n)]) for lo, n in ((0, 512), (512, 512), (1024, 1024))]
    cp_w = [fetch(wqkv_hbm.at[:, pl.ds(i * D, D)], wqkv_ref.at[i]) for i in range(3)]
    stages = [[cp_w[0], cp_x[0]],
              [cp_x[1], fetch(tw_hbm, tw_ref)],
              [cp_x[2], cp_w[2]],
              [fetch(dmat_hbm, dmat_ref), fetch(bx_hbm, bx_ref), cp_w[1], fetch(roots_hbm, roots_ref)],
              [fetch(wr_hbm, wr_ref), fetch(wi_hbm, wi_ref), fetch(nyq_hbm, nyq_ref)],
              [fetch(wo_hbm.at[pl.ds(0, 256)], wo_ref.at[pl.ds(0, 256)])],
              [fetch(wo_hbm.at[pl.ds(256, 256)], wo_ref.at[pl.ds(256, 256)])]]

    open_scope = []

    def mark(name):
        if cfg["scopes"]:
            if open_scope:
                open_scope.pop().__exit__(None, None, None)
            if name:
                open_scope.append(jax.named_scope(name))
                open_scope[-1].__enter__()

    def arrive(i):
        mark(f"wait{i}")
        for c in stages[i]:
            c.wait()
        mark(f"seg{i}")
        for c in (stages[i + cfg["late"]] if i + cfg["late"] < len(stages) else []):
            c.start()

    for stage in stages[:cfg["late"]]:
        for c in stage:
            c.start()

    def fill(i, c):
        for j in range(8):
            zero_ref[i * 8 + j] = 0
        return c

    lax.fori_loop(0, cfg["nz"] // 8, fill, 0)
    count = [0]

    def zero():
        count[0] += 1
        return zero_ref[count[0] % cfg["nz"]]

    qscale = DH ** -0.5 * math.log2(math.e)
    w_t = (wq_ref, None, wv_ref)
    qt = (qt_ref, qs_ref)
    qm_words, km_words, vt_words, xk_words = (ref.bitcast(U32) for ref in (qm_ref, km_ref, vt_ref, xk_ref))

    def transpose_weights(part):
        for j in range(4):
            w_t[part][0, 64 * j:64 * j + 64, :] = pltpu.bitcast(wqkv_ref[part, :, _tile(j)].T, U32)

    def project(part, x):
        return _dot_nt(pltpu.bitcast(w_t[part][zero()], BF16), x)

    def rows_of(t):
        return ax_ref[0, pl.ds(t * 128 if isinstance(t, int) else pl.multiple_of(t * 128, 128), 128), :]

    def project_q(u, j):
        y = project(0, rows_of(4 * u + j))
        q = (y * qscale).reshape(H, DH, 128)
        qt[j // 2][u, :, 0:DH, _tile(j % 2)] = q
        qm_ref[u, :, j] = q.astype(BF16)
        if j >= 2:
            first = qt[0][u + zero(), :, :, _tile(j % 2)]
            b11, b21, b12, b22 = first[:, :8], first[:, 8:], q[:, :8], q[:, 8:]
            t1 = b12 - b11
            t2 = b22 - t1
            for i, b in enumerate((b21 - t2, t1, t2, b22 - b12)):
                qt[1][u, :, 8 * i + 16:8 * i + 24, _tile(j % 2)] = b
        return y

    def gather_keys(r0, y):
        for r in range(r0, r0 + 32, 2):
            if r % 4 == 0:
                ax_ref[0, S:S + 8, 0:128] = y[12 * (r - r0):12 * (r - r0) + 8].astype(BF16)
                z = zero()
            x = jnp.concatenate([ax_ref[z, 8 * k:8 * k + 8, :].astype(F32) for k in key_order[r:r + 2]], axis=0)
            for c in range(4):
                xk_ref[c, 8 * r:8 * r + 16, :] = x[:, _tile(c)].astype(BF16)

    def project_k(t):
        r0, j = 64 * (t // 4), t % 4
        z = zero()
        x = jnp.concatenate([xk_words[c + z, 4 * r0:4 * r0 + 256, :] for c in range(4)], axis=1)
        y = _dot(pltpu.bitcast(x, BF16), wqkv_ref[1 + z, :, _tile(j)])
        lo = max(G - r0, 0)
        km_ref[j, 8 * (r0 + lo - G):8 * (r0 + 64 - G), :] = y[8 * lo:].astype(BF16)
        if lo:
            k = y[:8 * G].reshape(G // 2, 2, 8, 128)
            k1, k2 = k[:, 0].reshape(4 * G, 128), k[:, 1].reshape(4 * G, 128)
            s1 = k2 + pltpu.roll(k2, 120, 1)
            s2 = s1 - k1
            low = lax.broadcasted_iota(jnp.int32, k1.shape, 1) % DH < 8
            for i, a in enumerate((k1, jnp.where(low, s1, k2), jnp.where(low, s2, k1 - pltpu.roll(s2, 8, 1)), k1 - k2)):
                ks_ref[j, i] = a
        return y

    def project_v(t):
        y = project(2, rows_of(t))
        vt_ref[:, t] = y.reshape(H, DH, 128).astype(BF16)
        return y

    kh, kb = (kh0_ref, kh1_ref), (kb0_ref, kb1_ref)

    def prepare(h, slot, split):
        grp, shift = h // 8, (128 - DH * (h % 8)) % 128

        def mxu_rows(lo, hi, after):
            km_words[4, 0:8, :] = pltpu.bitcast(after, U32)
            kh[slot][0, lo:hi, :] = pltpu.roll(km_words[grp + zero(), lo:hi, :], shift, 1)

        def vpu_rows(i, lo, hi, after):
            ks_ref[4, 0, 0:8, :] = after
            src_ref[i, lo:hi, :] = pltpu.roll(ks_ref[grp + zero(), i, lo:hi, :], shift, 1)

        def vpu_plane(d, lo, hi, after):
            src_ref[0, 4 * G:4 * G + 8, :] = after
            i, col = ((0, 0), (0, 8), (2, 8), (1, 8), (1, 0), (2, 0), (3, 0))[d // 8]
            src = src_ref[i + zero(), lo:hi, :]
            kb[slot][0, d, lo:hi, :] = jnp.broadcast_to(src[:, col + d % 8:col + d % 8 + 1], (hi - lo, 128))

        def pieces(n, parts):
            cuts = [8 * (n * i // parts) for i in range(parts + 1)]
            return list(zip(cuts, cuts[1:]))

        steps = [functools.partial(vpu_rows, i, *cut) for i in range(4) for cut in pieces(G // 2, split)]
        steps += [functools.partial(mxu_rows, *cut) for cut in pieces(128 - G // 2, 5 * split)]
        return steps + [functools.partial(vpu_plane, d, *cut) for d in range(56) for cut in pieces(G // 2, split)]

    lane = lax.broadcasted_iota(jnp.int32, (128, 128), 1)
    even = lane % 2 == 0
    conj = jnp.where(even, 1.0, -1.0)
    spec = (fe_ref, fo_ref)

    def forward(a0, na):
        x = bx_ref[128 * a0:128 * (a0 + na), :].astype(F32)
        x0, x1, x2, x3 = (x[:, _tile(i)] for i in range(4))
        e0, e1, a, b = x0 + x2, x1 + x3, x0 - x2, x3 - x1
        z = zero()
        z0, z2 = _dot(e0 + e1, dmat_ref[z]), _dot(e0 - e1, dmat_ref[z + 1])
        t = _dot(a + b, dmat_ref[z + 2])
        re1, im1 = _dot(b, dmat_ref[z + 3]) + t, _dot(a, dmat_ref[z + 4]) + t
        for i in range(na):
            r = _tile(i)
            re_rows, im_rows = (pl.ds(XP * (a0 + i) + p, 128, stride=2) for p in range(2))
            im = pltpu.roll(jnp.where(even, z2[r], z0[r]), 127, 1)
            n_ref[:, a0 + i] = im.reshape(16, 8, 128)
            fe_ref[re_rows, :] = jnp.where(even, z0[r], z2[r])
            fe_ref[im_rows, :] = jnp.where(lane == 0, 0.0, im)
            fo_ref[re_rows, :] = re1[r]
            fo_ref[im_rows, :] = im1[r] * conj

    def backward(j):
        z = zero()
        re0, im0, re, im = (jnp.concatenate([ref[pl.ds(XP * a + 16 * j + p + z, 8, stride=2), :] for a in range(16)],
                                            axis=0) for ref in spec for p in range(2))
        im0 = pltpu.roll(im0, 1, 1)
        re0, im0 = jnp.where(even, re0, im0), jnp.where(even, im0, re0)
        if cfg["border"] == 0:
            t = _dot(re + im, dmat_ref[7])
            a, b = _dot(im, dmat_ref[8]) + t, _dot(re, dmat_ref[9]) + t
            u0, u2 = _dot(re0, dmat_ref[5]), _dot(im0, dmat_ref[6])
        else:
            t = jnp.concatenate([_dot((re + im)[r:r + 32], dmat_ref[7]) for r in range(0, 128, 32)], axis=0)
            a, b = _dot(im, dmat_ref[8]) + t, _dot(re, dmat_ref[9]) + t
            u0, u2 = _dot(re0, dmat_ref[5]), _dot(im0, dmat_ref[6])
        e0, e1 = u0 + u2, u0 - u2
        y = jnp.concatenate([e0 + a, e1 - b, e0 - a, e1 + b], axis=1).astype(BF16)
        for a in range(16):
            yb_ref[pl.ds(pl.multiple_of(128 * a + 8 * j, 8), 8), :] = y[8 * a:8 * a + 8]

    def filter_weights():
        for i, ref in enumerate((wr_ref, wi_ref)):
            for t in range(16):
                w = pltpu.bitcast(ref[0:256, _tile(t)], U32).T.reshape(8, 2, 8, 128)
                for hf in range(2):
                    w_ref[hf, i, 8 * t:8 * t + 8] = w[:, hf]

    pace = dict(jobs=[], clock=0.0, rate=1.0, done=0, rows=None)

    def start(jobs, ops, span, extra=(), lead=cfg['lead']):
        pace.update(extra=list(extra), due=0.0, gap=512.0 * (span - 0.5) / max(len(extra), 1))
        pace.update(jobs=list(jobs), clock=-lead, rate=ops / (512.0 * span + lead), done=0)

    def finish():
        while pace["jobs"]:
            pace["jobs"].pop(0)()
        assert not pace["extra"]

    def gate(spare, ops):
        while pace["jobs"] and pace["clock"] >= 512 * pace["done"]:
            pace["rows"] = pace["jobs"].pop(0)()
            pace["done"] += 1
        r = int(pace["clock"]) - 512 * (pace["done"] - 1)
        if pace["done"] and r < 512:
            row = pace["rows"][r // 8 * 8:r // 8 * 8 + 8]
            spare[...] = pltpu.bitcast(row, spare.dtype)
            if pace["extra"] and pace["clock"] >= pace["due"]:
                pace["extra"].pop(0)(row)
                pace["due"] += pace["gap"]
        pace["clock"] += ops / pace["rate"]
        return zero()

    def data(odd, stride, rows, swap, ops):
        ref = spec[odd]
        z = gate(ref.at[pl.ds(16 * XP, 8)], ops)
        return [tuple(ref[pl.ds(r + (p ^ swap) + z, 8, stride=stride), :] for p in range(2)) for r in rows]

    def put(odd, stride, rows, vals, swap):
        z = zero() if cfg["oput"] else 0
        for r, val in zip(rows, vals):
            for p in range(2):
                spec[odd][pl.ds(r + (p ^ swap) + z, 8, stride=stride), :] = val[p]

    def rotate(vals, ks, ops=0):
        z = gate(roots_ref.at[0, pl.ds(128, 8), pl.ds(0, 128)], ops + sum(0 if k == 0 else 4 if k % 32 == 16 else 6 for k in ks))
        out = []
        for (re, im), k in zip(vals, ks):
            c, s = (jnp.broadcast_to(roots_ref[z, k:k + 1, _tile(p)], (8, 128)) for p in range(2))
            if k == 0:
                out.append((re, im))
            elif k % 64 == 16:
                out.append(((re + im) * c, (im - re) * c))
            elif k % 64 == 48:
                out.append(((re - im) * c, (re + im) * c))
            else:
                out.append(_cmul((re, im), c, s))
        return out

    def second_half(cols, k1):
        ks = [0 if n * k1 == 4 else 8 * n * k1 for n in range(4)]
        return _dft4(rotate([col[k1] for col in cols], ks, 16), k1 == 2)

    def twiddle(vals, j, f1s):
        z = gate(twb_ref.at[0, 0, 0], 6 * sum(f1 > 0 for f1 in f1s))
        return [_cmul(v, twb_ref[j + z, f1, 0], twb_ref[j + z, f1, 1]) if f1 else v
                for v, f1 in zip(vals, f1s)]

    def outer(j, odd):
        rows = [XP * a + 16 * j for a in range(16)]
        cols = [_dft4(data(odd, 2, rows[n::4], 0, 16)) for n in range(4)]
        for k1 in range(4):
            put(odd, 2, rows[k1::4], twiddle(second_half(cols, k1), j, range(k1, 16, 4)), 0)

    def outer_inverse(j, odd):
        rows = [XP * a + 16 * j for a in range(16)]
        cols = [_dft4(twiddle(data(odd, 2, rows[n::4], 1, 16), j, range(n, 16, 4))) for n in range(4)]
        for k1 in range(4):
            out = []
            for a, (im, re) in zip(range(k1, 16, 4), second_half(cols, k1)):
                if odd:
                    out.append((re, im * conj[:8]))
                else:
                    out.append((re, jnp.where(lane[:8] == 0, n_ref[j, a], im)))
            put(odd, 2, rows[k1::4], out, 0)

    def inner(hf, e, odd, inverse):
        rows = [8 * XP * hf + 2 * b for b in range(e, 128, 16)]
        cols = []
        for n in range(2):
            vals = data(odd, XP, rows[n::2], inverse, 0 if inverse else 16)
            cols.append(_dft4(rotate(vals, [e * g for g in range(n, 8, 2)], 16) if inverse else vals))
        for k1 in range(2):
            lo, hi = cols[1][k1::2]
            if k1:
                lo, hi = rotate([lo, hi], [16, 48], 16)
            (y0, y2), (y1, y3) = _pm(cols[0][k1], lo), _pm(cols[0][k1 + 2], hi, k1 == 0)
            out = [y0, y1, y2, y3]
            put(odd, XP, rows[k1::2], out if inverse else rotate(out, [e * g for g in range(k1, 8, 2)]), inverse)

    def centre(hf, g1, odd):
        rows = [8 * XP * hf + 2 * b for b in range(16 * g1, 16 * g1 + 16)]
        cols = [_dft4(data(odd, XP, rows[n::4], 0, 16)) for n in range(4)]
        back = []
        for k1 in range(4):
            vals = []
            for g2, val in zip(range(k1, 16, 4), second_half(cols, k1)):
                if g2 // 4 % 2 == 0:
                    z = gate(w_ref.at[0, 0, 128], 16 if g2 < 4 else 32)
                wr, wi = (pltpu.bitcast(w & np.uint32(0xFFFF0000) if odd else w << 16, F32)
                          for w in (w_ref[hf + z, 0, g1 + 8 * g2], w_ref[hf + z, 1, g1 + 8 * g2]))
                vals.append(_cmul(val, wr, wi)[::-1])
            back.append(_dft4(vals))
        for k1 in range(4):
            put(odd, XP, rows[k1::4], second_half(back, k1), 1)

    nyq = {}

    def nyquist(step):
        twr, twi = tw_ref[0:128, :], tw_ref[128:256, :]
        if step == 0:
            zn = jnp.concatenate([n_ref[:, t].reshape(128, 128).T[0:1] for t in range(16)], axis=0)
            t = _dot(nyq_ref[0:256, 0:16], zn)
            tr, ti = t[:128], t[128:]
            nyq[0] = jnp.concatenate([tr * twr - ti * twi, tr * twi + ti * twr], axis=1)
        elif step == 1:
            wr, wi = (jnp.concatenate([ref[256:257, _tile(t)].astype(F32) for t in range(16)], axis=0)
                      for ref in (wr_ref, wi_ref))
            zf = _dot_nt(jnp.concatenate([nyq_ref[512:544, :], nyq_ref[560:592, :]], axis=1), nyq[0])
            zr, zi = zf[:16], zf[16:]
            nyq[1] = jnp.concatenate([zr * wr - zi * wi, zr * wi + zi * wr], axis=0)
        elif step == 2:
            t = _dot(nyq_ref[256:512, 0:32], nyq[1])
            tr, ti = t[:128], t[128:]
            nyq[2] = jnp.concatenate([tr * twr + ti * twi, ti * twr - tr * twi], axis=1)
        else:
            yn = _dot_nt(jnp.concatenate([nyq_ref[544:560, :], nyq_ref[592:608, :]], axis=1), nyq[2])
            for t in range(16):
                n_ref[:, t] = jnp.broadcast_to(yn[t:t + 1], (128, 128)).T.reshape(16, 8, 128)

    cp_w[0].wait()
    transpose_weights(0)
    stages[0].pop(0)
    arrive(0)
    if "pre" not in skip:
        for t in range(4):
            project_q(0, t)
    arrive(1)
    if "pre" not in skip:
        for f1 in range(1, 16):
            tw = jnp.broadcast_to(tw_ref[...][:, f1:f1 + 1], (256, 128)).reshape(2, 16, 8, 128)
            for p in range(2):
                twb_ref[:, f1, p] = tw[p]
        for t in range(4):
            project_q(1, t)
    arrive(2)
    if "pre" not in skip:
        transpose_weights(2)
        for t in range(8):
            gather_keys(32 * t, project_q(2 + t // 4, t % 4))
    arrive(3)
    jobs = [functools.partial(project_k, t) for t in range(16)] + [functools.partial(project_v, t) for t in range(16)]
    n3, n4 = cfg["njobs"]
    if "pre" not in skip:
        for a in range(0, 16, cfg["fwd_n"]):
            forward(a, cfg["fwd_n"])
        start(jobs[:n3], 32 * 258, n3 - cfg['slack3'], lead=0)
        for j in range(16):
            for odd in range(2):
                outer(j, odd)
        finish()
    arrive(4)
    if "pre" not in skip:
        filter_weights()

        def job(t):
            if t - 1 in cfg["nyq_at"]:
                nyquist(cfg["nyq_at"].index(t - 1))
            return jobs[n3 + t]()

        start([functools.partial(job, t) for t in range(n4)], 64 * 94, n4 - cfg['slack4'])
        for hf in range(2):
            for e in range(16):
                for odd in range(2):
                    inner(hf, e, odd, 0)
        finish()
    if "pre" not in skip:
        steps = prepare(0, 0, cfg["split0"])
        steps = steps[:4 * cfg["split0"]] + steps[9 * cfg["split0"]:] + steps[4 * cfg["split0"]:9 * cfg["split0"]]
        if not cfg["prep0"]:
            steps = []
        rest = jobs[n3 + n4:]
        for hf in range(2):
            if cfg["merge"]:
                if hf == 0:
                    arrive(5)
                    arrive(6)
                    start(rest, 32 * 464 + 64 * 94 + 258 * cfg["hpi"], len(rest) - cfg["slack"], steps)
            else:
                arrive(5 + hf)
                mine = rest[:len(rest) // 2] if hf == 0 else rest[len(rest) // 2:]
                start(mine, 16 * 464 + 32 * 94 + 258 * cfg["hpi"] * hf, len(mine) - (cfg["slack"] if hf else 0.3),
                      steps[:len(steps) // 2] if hf == 0 else steps[len(steps) // 2:])
            for g1 in range(8):
                for odd in range(2):
                    centre(hf, g1, odd)
            for e in range(16):
                for odd in range(2):
                    inner(hf, e, odd, 1)
            for j in range(cfg["hpi"] // 2 * hf):
                for odd in range(2):
                    outer_inverse(j, odd)
            if hf or not cfg["merge"]:
                finish()
    else:
        arrive(5)
        arrive(6)
    mark("attn")

    HPI = cfg["hpi"]
    ops = _mxu_order(plan, cfg["lag"], 4 * HPI)

    def vpu_scores(h, slot, t0, idx):
        z = zero()

        def prod(i, s=None):
            for d in range(8):
                ref, row = (qt[0], 8 * i + d) if i < 2 else (qt[1], 8 * i + d - 8)
                q = jnp.concatenate([jnp.broadcast_to(ref[t0 // 4, h + z, row:row + 1, _tile(c)], (8, 128))
                                     for c in range(2)], axis=1)
                term = jnp.concatenate([kb[slot][z, 8 * i + d, idx * 8:idx * 8 + 8, :]] * 2, axis=1) * q
                s = term if s is None else s + term
            return s

        p1, p5 = prod(0), prod(4)
        c11, u2 = prod(1, p1), prod(5, p1)
        u3 = prod(6, u2)
        if cfg["form"] == 0:
            c12, c21 = prod(2, u2 + p5), prod(3, u3)
        elif cfg["form"] == 1:
            c12, c21 = prod(2, p5) + u2, prod(3, u3)
        elif cfg["form"] == 2:
            c12, c21 = prod(2, u2) + p5, prod(3, u3)
        else:
            c12, c21 = prod(2, p5) + u2, prod(3) + u3
        return jnp.concatenate([c11, c12], axis=1), jnp.concatenate([c21, u3 + p5], axis=1)

    def heads(it, c):
        probs, scores, acc, den, seen = {}, {}, {}, {}, []
        for n, op in enumerate(ops):
            u = op[1]
            slot, t0 = (u // 4) % 2, (u % 4) * 4
            h = it * HPI + u // 4
            if n == len(ops) - cfg["back_at"] and cfg["tail"]:
                for j in range(HPI // 2):
                    backward(it * (HPI // 2) + j)
            if op[0] == "qk":
                lo, hi = op[2:]
                z = zero()
                keys = pltpu.bitcast(kh[slot][z, lo * 8:hi * 8, 0:DH], BF16)
                q = pltpu.bitcast(jnp.concatenate([qm_words[t0 // 4, h + z, j] for j in range(4)], axis=1), BF16)
                p = jnp.exp2(_dot(keys, q))
                for r in range(2 * (hi - lo)):
                    probs[u, 2 * lo + r] = p[r * 8:(r + 1) * 8]
                continue
            blk = op[2]
            if u % 4 == 0 and blk == 0:
                steps = prepare(jnp.minimum(h + 1, H - 1), 1 - slot, cfg['split'])
                total = len(steps)
            tile = []
            for on_vpu, i in plan[16 * blk:16 * blk + 16]:
                if on_vpu and i % 2 == 0:
                    scores[u, i], scores[u, i + 1] = vpu_scores(h, slot, t0, i // 2)
                tile.append(jnp.exp2(scores.pop((u, i))) if on_vpu else probs.pop((u, i)))
            for i, p in enumerate(tile):
                den[u] = den[u] + p if u in den else p
                seen.append(den[u])
                progress = ((u % 4) * 256 + blk * 16 + i + 1 - cfg["delay"]) / (16.0 * cfg["prep_span"])
                if steps and total - len(steps) < progress * total and not plan[16 * blk + i][0]:
                    steps.pop(0)(p[:, _tile(cfg['gcol'])] if cfg['gcol'] < 4 else den[u][:, _tile(cfg['gcol'] - 4)])
            vals = pltpu.bitcast(vt_words[h + zero(), blk], BF16)
            o = _dot(vals, jnp.concatenate(tile[::-1], axis=0))
            acc[u] = o + acc[u] if u in acc else o
            if blk == 15:
                o, l = acc.pop(u), den.pop(u)
                for j in range(4):
                    ot_ref[t0 + j, h] = o[:, _tile(j)]
                    den_ref[t0 + j, pl.ds(h, 8, stride=DP), :] = l[:, _tile(j)]
        if cfg["tail"] == 1:
            start([], 1, 1)
            for odd in range(2):
                spec[odd][16 * XP:16 * XP + 8, :] = seen[-cfg["tgate"][odd]][:, 0:128]
            twb_ref[0, 0, 0] = seen[-cfg["tgate"][0]][:, 0:128]
            for j in range(HPI // 2):
                for odd in range(2):
                    outer_inverse(((it + 1) * (HPI // 2) + j) % 16, odd)
        return c

    if "attn" not in skip:
        lax.fori_loop(0, H // HPI, heads, 0)
    else:
        def keep(h, c):
            t = h % 16
            x = qt_ref[t // 4, h, :, 0:128] + qs_ref[t // 4, h, 0:16, 0:128] + pltpu.bitcast(km_words[t % 4, 0:16], F32) + pltpu.bitcast(vt_words[h, t], BF16).astype(F32)
            x = x + ks_ref[t % 4, 0, 0:16] + kb[0][0, t, 0:16] + n_ref[t, 0:2].reshape(16, 128)
            x = x + pltpu.bitcast(kh[0][zero(), 0:16], F32) + fe_ref[pl.ds(h * 16, 16), :] + fo_ref[pl.ds(h * 16, 16), :]
            ot_ref[t, h] = x
            den_ref[t, 0:8] = pltpu.bitcast(qm_words[t // 4, h, 0], F32)
            return c
        lax.fori_loop(0, H, keep, 0)

    mark('post')
    cp_yb = pltpu.make_async_copy(yb_ref, out_hbm.at[:, pl.ds(D, D)], out_sem.at[0])
    cp_yb.start()
    edges = np.cumsum((0,) + cfg["out_rows"]).tolist()
    cp_ya = [pltpu.make_async_copy(ya_ref.at[pl.ds(lo, hi - lo)], out_hbm.at[pl.ds(lo, hi - lo), pl.ds(0, D)],
                                   out_sem.at[1 + i]) for i, (lo, hi) in enumerate(zip(edges, edges[1:]))]
    bad = jnp.zeros((H, 128), F32)
    for cp, lo, hi in zip(cp_ya, edges, edges[1:]):
        if "post" in skip:
            z = zero()
            x = ot_ref[z, 0] + den_ref[z, 0:16] + kb[1][z, 0, 0:16] + pltpu.bitcast(kh[1][z, 0:16], F32)
            ya_ref[0:16, 0:128] = x.astype(BF16)
            cp.start()
            continue
        rows = []
        for t in range(lo // 128, hi // 128):
            l = den_ref[t, 0:H, :]
            for r in range(1, 8):
                l = l + den_ref[t, DP * r:DP * r + H, :]
            bad = jnp.where((l >= 2.0 ** -20) & (l <= 2.0 ** 40), bad, 1.0)
            inv_ref[t] = 1.0 / l
            o = [ot_ref[t, h] * jnp.broadcast_to(inv_ref[t, h:h + 1, :], (DH, 128)) for h in range(H)]
            rows.append(jnp.concatenate(o, axis=0).astype(BF16).T)
        ya_ref[lo:hi, :] = _dot(jnp.concatenate(rows, axis=0), wo_ref[...]).astype(BF16)
        cp.start()
    unsafe = jnp.max(bad) > 0.0
    mark('drain')
    for cp in cp_ya + [cp_yb]:
        cp.wait()
    mark(None)

    @pl.when(unsafe)
    def _():
        def group(grp, c):
            def keys_values(i, c):
                rows = pl.ds(pl.multiple_of(i * 256, 256), 256)
                for part in range(3):
                    col = pl.multiple_of(grp * 128, 128)
                    kf_ref[part, rows, :] = _dot(ax_ref[0, rows, :], wqkv_ref[part, :, pl.ds(col, 128)])
                of_ref[grp, rows, :] = jnp.zeros((256, 128), F32)
                return c

            lax.fori_loop(0, S // 256, keys_values, 0)

            def block(i, c):
                j, rows = i % 8, pl.ds(pl.multiple_of((i // 8) * 128, 128), 128)
                mine = lax.broadcasted_iota(jnp.int32, (S, 128), 1) // DH == j
                q = jnp.where(mine[:128], kf_ref[0, rows, :] * qscale, 0.0)
                s = _dot_nt(q, jnp.where(mine, kf_ref[1], 0.0))
                p = jnp.exp2(s - jnp.max(s, axis=1, keepdims=True))
                o = _dot(p / jnp.sum(p, axis=1, keepdims=True), kf_ref[2])
                of_ref[grp, rows, :] = jnp.where(mine[:128], o, of_ref[grp, rows, :])
                return c

            return lax.fori_loop(0, 8 * 16, block, c)

        lax.fori_loop(0, 4, group, 0)

        def project_out(i, c):
            rows = pl.ds(pl.multiple_of(i * 256, 256), 256)
            o = jnp.concatenate([of_ref[j, rows, :] for j in range(4)], axis=1)
            ya_ref[rows, :] = _dot(o, wo_ref[...]).astype(BF16)
            return c

        lax.fori_loop(0, S // 256, project_out, 0)
        cp = pltpu.make_async_copy(ya_ref, out_hbm.at[:, pl.ds(0, D)], out_sem.at[0])
        cp.start()
        cp.wait()


def make(**over):
    cfg = dict(CFG, **over)
    g = cfg["g"]
    vmem = pltpu.VMEM
    scratch = [
        vmem((1, S + 16, D), BF16), vmem((3, D, D), BF16), vmem((D, D), BF16), vmem((S, D), BF16),
        vmem((D // 2 + 1, S), BF16), vmem((D // 2 + 1, S), BF16),
        vmem(_DMAT.shape, BF16), vmem(_NYQ.shape, BF16), vmem(_TW.shape, F32), vmem(_ROOTS.shape, F32),
        vmem((1, D // 2, D), U32), vmem((1, D // 2, D), U32),
        vmem((4, H, DH, 256), F32), vmem((4, H, 4, DH, 128), BF16), vmem((4, H, 48, 256), F32),
        vmem((4, S, 128), BF16), vmem((5, S, 128), BF16), vmem((5, 4, 4 * g, 128), F32), vmem((H, 16, DH, 128), BF16), vmem((16, H, DH, 128), F32),
        vmem((16, 8 * DP, 128), F32), vmem((16, H, 128), F32),
        vmem((1, S // 2, 128), U32), vmem((1, S // 2, 128), U32),
    ] + [vmem((1, 56, 4 * g, 128), F32)] * 2 + [vmem((4, 256, 128), F32),
        vmem((16 * XP + 32, 128), F32), vmem((16 * XP + 32, 128), F32), vmem((16, 16, 2, 8, 128), F32),
        vmem((2, 2, 132, 8, 128), U32), vmem((16, 16, 8, 128), F32),
        vmem((S, D), BF16), vmem((S, D), BF16), vmem((3, S, 128), F32), vmem((4, S, 128), F32),
        pltpu.SMEM((cfg["nz"],), jnp.int32),
        pltpu.SemaphoreType.DMA((15,)),
        pltpu.SemaphoreType.DMA((len(cfg["out_rows"]) + 1,)),
    ]

    def fn(A_x, A_wqkv, A_wo, B_x, B_w_r, B_w_i):
        out = pl.pallas_call(
            functools.partial(_kernel, cfg),
            out_shape=jax.ShapeDtypeStruct((S, 2 * D), BF16),
            in_specs=[pl.BlockSpec(memory_space=pl.ANY)] * 10,
            out_specs=pl.BlockSpec(memory_space=pl.ANY),
            scratch_shapes=scratch,
            compiler_params=pltpu.CompilerParams(vmem_limit_bytes=110 * 1024 * 1024, flags=cfg["flags"]),
            name="mha_gfnet",
        )(A_x.reshape(S, D), A_wqkv, A_wo, B_x.reshape(S, D), B_w_r.T, B_w_i.T, _DMAT, _NYQ, _TW, _ROOTS)
        return out.reshape(1, S, 2 * D)

    return jax.jit(fn)


_FN = make()


@jax.jit
def pallas_concat_heads__mha_block__spectral_gfnet__prompt_kernel(A_x, A_wqkv, A_wo, B_x, B_w_r, B_w_i):
    return _FN(A_x, A_wqkv, A_wo, B_x, B_w_r, B_w_i)
```

```python
import functools
import math

import jax
import jax.numpy as jnp
import numpy as np
from jax import lax
import jax.experimental.pallas as pl
import jax.experimental.pallas.tpu as pltpu

S, D, H, DH = 2048, 512, 32, 16
F32, BF16, U32 = jnp.float32, jnp.bfloat16, jnp.uint32

QSCALE = DH ** -0.5 * math.log2(math.e)
RANGE = 32.0
GRID = 2.0 ** -8
MAGIC = 1.5 * 2.0 ** 23 * GRID
LOW = GRID / (2.0 * RANGE)

FFT_PITCH = 260
SUM_PITCH = 36
N_ZEROS = 256
LOOKAHEAD = 8


def _constants():
    n = np.arange(128)[:, None]
    m = np.arange(64)[None, :]

    def cs(num, den):
        ang = 2.0 * np.pi * (num % den) / den
        return np.cos(ang), -np.sin(ang)

    def interleave(re, im, shift):
        return np.roll(np.stack([re, im], axis=2).reshape(128, 128), shift, axis=1)

    mats = [interleave(*cs(n * 4 * m, D), 0), interleave(*cs(n * (4 * m + 2), D), 1)]
    for first in (1, 5):
        mat = np.zeros((128, 128))
        for lane in range(128):
            k = 2 * lane + 1
            if first in (k % 8, -k % 8):
                c, s = cs(n[:64, 0] * (k if k % 8 == first else D - k), D)
                mat[:, lane] = np.concatenate([c, -s])
                mat[:, (lane + 2) % 128] = np.concatenate([s, c]) * (1.0 if k % 8 == first else -1.0)
        mats.append(mat)
    mats += [mat.T * (2.0 / (S * D)) for mat in mats]
    mats[0][:, 1] = (-1.0) ** np.arange(128)
    mats[4][0], mats[4][1] = 1.0 / (S * D), mats[0][:, 1] / (S * D)

    c, s = cs(n * np.arange(16)[None, :], 16)
    nyquist = np.zeros((640, 128))
    nyquist[:256, :16] = np.concatenate([c, s])
    nyquist[256:512, :32] = np.block([[c, s], [-s, c]])
    nyquist[512:608] = np.concatenate([c.T, s.T, c.T, -s.T, c.T, s.T])
    twiddles = np.concatenate(cs(n * n.T, S))
    roots = np.zeros((1, 144, 256))
    roots[0, :128, :128], roots[0, :128, 128:] = cs(n, 128)
    return (np.stack(mats).astype(jnp.bfloat16), nyquist.astype(jnp.bfloat16),
            twiddles.astype(np.float32), roots.astype(np.float32))


_DFT, _NYQUIST, _TWIDDLES, _ROOTS = _constants()


def _cmul(z, c, s):
    re, im = z
    return re * c - im * s, re * s + im * c


def _butterfly(a, b, quarter=False):
    (ar, ai), (br, bi) = a, b
    if quarter:
        return (ar + bi, ai - br), (ar - bi, ai + br)
    return (ar + br, ai + bi), (ar - br, ai - bi)


def _dft4(x, quarter=False):
    s0, d0 = _butterfly(x[0], x[2], quarter)
    s1, d1 = _butterfly(x[1], x[3])
    (y0, y2), (y1, y3) = _butterfly(s0, s1), _butterfly(d0, d1, True)
    return [y0, y1, y2, y3]


def _dot(a, b):
    return lax.dot_general(a, b, (((1,), (0,)), ((), ())), preferred_element_type=F32)


def _dot_nt(a, b):
    return lax.dot_general(a, b, (((1,), (1,)), ((), ())), preferred_element_type=F32)


def _tile(j):
    return slice(j * 128, (j + 1) * 128)


def _block(i, size):
    return pl.ds(i * size if isinstance(i, int) else pl.multiple_of(i * size, size), size)


def _kernel(ax_hbm, wqkv_hbm, wo_hbm, bx_hbm, wr_hbm, wi_hbm, dft_hbm, nyq_hbm, tw_hbm, roots_hbm, out_hbm,
            ax_ref, wqkv_ref, wo_ref, bx_ref, wf_ref, dft_ref, nyq_ref, tw_ref, roots_ref,
            wq_ref, wk_ref, wv_ref, q_ref, kt_ref, v0_ref, v1_ref, k0_ref, k1_ref, sq_ref, peak_ref,
            o_ref, den_ref, inv_ref, u_ref, f_ref, t_ref, g_ref, twb_ref, w_ref, n_ref, ya_ref, yb_ref, zero_ref, sems):
    def x_tiles(lo, hi):
        rows = pl.ds(128 * lo, 128 * (hi - lo))
        return ax_hbm.at[rows], ax_ref.at[rows]

    def w_part(i, lo=0, n=D):
        return wqkv_hbm.at[:, pl.ds(i * D + lo, n)], wqkv_ref.at[i, :, pl.ds(lo, n)]

    stages = [[w_part(0, 0, 256)], [x_tiles(0, 3)], [x_tiles(3, 4), w_part(0, 256, 256)],
              [x_tiles(4, 8), (tw_hbm, tw_ref)], [x_tiles(8, 14)], [x_tiles(14, 16), w_part(1)],
              [(dft_hbm, dft_ref), (bx_hbm, bx_ref.at[0, pl.ds(0, S)])],
              [w_part(2), (roots_hbm, roots_ref), (wr_hbm, wf_ref.at[0]), (wi_hbm, wf_ref.at[1]),
               (nyq_hbm, nyq_ref), (wo_hbm, wo_ref)]]
    stages = [[pltpu.make_async_copy(src, dst, sems.at[i]) for src, dst in stage] for i, stage in enumerate(stages)]
    out_sem = sems.at[len(stages)]
    for stage in stages:
        for copy in stage:
            copy.start()

    def arrive():
        for copy in stages.pop(0):
            copy.wait()

    def fill(i, carry):
        for j in range(8):
            zero_ref[i * 8 + j] = 0
        return carry

    lax.fori_loop(0, N_ZEROS // 8, fill, 0)
    pace = {"zeros": 0}

    def zero():
        pace["zeros"] += 1
        return zero_ref[pace["zeros"] % N_ZEROS]

    def start(stream, ops, ticks, first=0.0):
        pace.update(stream=stream, clock=first, rate=ops / ticks, tick=-1)

    def gate(spare, ops):
        while pace["tick"] < int(pace["clock"]):
            pace["result"] = next(pace["stream"])
            pace["tick"] += 1
        spare[...] = pace["result"]()
        pace["clock"] += ops / pace["rate"]
        return zero()

    def finish(stream):
        for _ in stream:
            pass

    w_refs, k_refs, v_refs = (wq_ref, wk_ref, wv_ref), (k0_ref, k1_ref), (v0_ref, v1_ref)
    q_words, kt_words = q_ref.bitcast(U32), kt_ref.bitcast(U32)

    def transpose_weights(part, lo=0, hi=4):
        for j in range(lo, hi):
            w_refs[part][0, 64 * j:64 * j + 64, :] = pltpu.bitcast(wqkv_ref[part, :, _tile(j)].T, U32)

    def project(part, t, lo=0, hi=H):
        if part == 1:
            groups = [32 * (t // 2) + 16 * (r // 8) + 15 - 2 * (r % 8) - t % 2 for r in range(16)]
            x = jnp.concatenate([ax_ref[8 * g:8 * g + 8, :].astype(F32) for g in groups], axis=0).astype(BF16)
        else:
            x = ax_ref[_block(t, 128), :]
        y = _dot_nt(pltpu.bitcast(w_refs[part][zero(), 8 * lo:8 * hi, :], BF16), x)
        z = y.reshape(hi - lo, DH, 128)
        if part == 2:
            if lo == 0:
                v0_ref[:, t] = z[:16].astype(BF16)
            v1_ref[max(lo - 16, 0):hi - 16, t] = z[max(16 - lo, 0):].astype(BF16)
            peak_ref[2, 0:8] = jnp.maximum(peak_ref[2, 0:8], jnp.max(jnp.abs(y).reshape(-1, 8, 128), axis=0))
            return y
        if part == 0:
            q_ref[lo:hi, t] = (z * QSCALE).astype(BF16)
        else:
            kt_ref[0:H, t] = (z * LOW if t % 2 else z).astype(BF16)
        square = z * z
        square = square[:, :8] + square[:, 8:]
        for h in range(lo, hi):
            sq_ref[16 * part + t, pl.ds(h, 8, stride=SUM_PITCH), :] = square[h - lo]
        return y

    def projections(jobs, steps):
        steps, tick = sorted(steps, key=lambda step: step[0]), -1
        for job in jobs:
            y = project(*job)
            for r in range(0, y.shape[0], 8):
                tick += 1
                while steps and steps[0][0] <= tick:
                    steps.pop(0)[1](y[r:r + 8])
                yield lambda: y[r:r + 8]
        assert not steps

    def spread(steps, lo, hi):
        return [(64 * (lo + (hi - lo) * i / len(steps)), step) for i, step in enumerate(steps)]

    def sublane_sum(ref, t):
        return functools.reduce(jnp.add, [ref[t, SUM_PITCH * r:SUM_PITCH * r + H, :] for r in range(8)])

    row = lax.broadcasted_iota(jnp.int32, (DH, 128), 0)
    magic = pltpu.bitcast(jnp.where(row == 0, MAGIC, jnp.where(row == 8, -MAGIC, 0.0)).astype(BF16), U32)
    ones = pltpu.bitcast(jnp.ones((DH, 512), BF16), U32)

    def pair_keys(half, h, t, after):
        kt_words[H, 0] = pltpu.bitcast(after, U32)
        hz = 16 * half + h + zero()
        both = jnp.concatenate([kt_words[hz, 2 * t], magic, kt_words[hz, 2 * t + 1]], axis=0)
        k_refs[half][h, 64 * t:64 * t + 64, 0:48] = pltpu.bitcast(pltpu.bitcast(both, BF16).T, U32)

    def pairs(lo, hi):
        return [functools.partial(pair_keys, 0, h, t) for t in range(lo, hi) for h in range(16)]

    lane = lax.broadcasted_iota(jnp.int32, (128, 128), 1)
    left = lane < 64
    own = (lane % 2 == 0, (lane + 1) % 4 < 2)
    dft_words, u_words = dft_ref.bitcast(U32), u_ref.bitcast(U32)

    def dft_matrix(i):
        return pltpu.bitcast(dft_words[i], BF16)

    def split_rows(r, after):
        bx_ref[0, S:S + 8, 0:128] = after.astype(BF16)
        x = bx_ref[zero(), r:r + 16, :].astype(F32)
        x0, x1, x2, x3 = (x[:, _tile(i)] for i in range(4))
        e0, e1, o0, o1 = x0 + x2, x1 + x3, x0 - x2, x3 - x1
        p = jnp.where(left[:16], o0, pltpu.roll(o1, 64, 1))
        q = jnp.where(left[:16], pltpu.roll(o0 + o1, 64, 1), o1 - o0) * math.sqrt(0.5)
        for i, val in enumerate((e0 + e1, e0 - e1, p + q, p - q)):
            u_ref[i, r:r + 16, :] = val.astype(BF16)

    def forward(a, _):
        z = zero()
        y = [_dot(pltpu.bitcast(u_words[i, 64 * a:64 * a + 64, :], BF16), dft_matrix(z + i)) for i in range(4)]
        for odd in range(2):
            im = pltpu.roll(jnp.where(own[odd], y[2 * odd + 1], y[2 * odd]), 127 - odd, 1)
            if not odd:
                n_ref[:, a] = im.reshape(16, 8, 128)
                im = jnp.where(lane == 0, 0.0, im)
            f_ref[odd, pl.ds(FFT_PITCH * a, 128, stride=2), :] = jnp.where(own[odd], y[2 * odd], y[2 * odd + 1])
            f_ref[odd, pl.ds(FFT_PITCH * a + 1, 128, stride=2), :] = im

    def backward(j):
        z = zero()
        y = [_dot(g_ref[z + i], dft_matrix(z + 4 + i)) for i in range(4)]
        e0, e1, p, q = y[0] + y[1], y[0] - y[1], y[2] + y[3], (y[2] - y[3]) * math.sqrt(0.5)
        turned = pltpu.roll(q, 64, 1)
        o0, o1 = jnp.where(left, p, turned - q), jnp.where(left, pltpu.roll(p, 64, 1), turned + q)
        y = jnp.concatenate([e0 + o0, e1 - o1, e0 - o0, e1 + o1], axis=1).astype(BF16)
        yb_ref[:, _block(j, 8), :] = y.reshape(16, 8, D)

    def filtered_rows(i):
        rows = _block(i, 32)
        return pltpu.make_async_copy(yb_ref.at[:, rows], out_hbm.at[:, rows, pl.ds(D, D)], out_sem)

    def filter_weights(i, t, after):
        wf_ref[2, 0:8, 0:128] = after.astype(BF16)
        w = pltpu.bitcast(wf_ref[i + zero(), 0:256, _tile(t)], U32).T.reshape(8, 2, 8, 128)
        for half in range(2):
            w_ref[2 * half, i, 8 * t:8 * t + 8] = pltpu.bitcast(w[:, half] << 16, F32)
            w_ref[2 * half + 1, i, 8 * t:8 * t + 8] = pltpu.bitcast(w[:, half] & np.uint32(0xFFFF0000), F32)

    def load(odd, stride, rows, swap, ops):
        z = odd + gate(f_ref.at[0, pl.ds(16 * FFT_PITCH, 8)], ops)
        return [tuple(f_ref[z, pl.ds(r + (p ^ swap), 8, stride=stride), :] for p in range(2)) for r in rows]

    def store(odd, stride, rows, vals, swap):
        z = odd + zero()
        for r, val in zip(rows, vals):
            for p in range(2):
                f_ref[z, pl.ds(r + (p ^ swap), 8, stride=stride), :] = val[p]

    def park(slot, n, vals):
        for k, val in enumerate(vals):
            for p in range(2):
                t_ref[slot, k, n, p] = val[p]

    def parked(slot, k):
        z = slot + gate(t_ref.at[2, 0, 0, 0], 0)
        return [(t_ref[z, k, n, 0], t_ref[z, k, n, 1]) for n in range(4)]

    def rotate(vals, ks, ops=0):
        z = gate(roots_ref.at[0, pl.ds(128, 8), pl.ds(0, 128)],
                 ops + sum(0 if k == 0 else 4 if k % 32 == 16 else 6 for k in ks))
        out = []
        for (re, im), k in zip(vals, ks):
            if k == 0:
                out.append((re, im))
                continue
            c = jnp.broadcast_to(roots_ref[z, k:k + 1, _tile(0)], (8, 128))
            if k % 64 == 16:
                out.append(((re + im) * c, (im - re) * c))
            elif k % 64 == 48:
                out.append(((re - im) * c, (re + im) * c))
            else:
                out.append(_cmul((re, im), c, jnp.broadcast_to(roots_ref[z, k:k + 1, _tile(1)], (8, 128))))
        return out

    def dft16_row(vals, k):
        return _dft4(rotate(vals, [0 if n * k == 4 else 8 * n * k for n in range(4)], 16), k == 2)

    def twiddle(vals, j, f1s):
        z = j + gate(twb_ref.at[0, 0, 0], 6 * sum(f1 > 0 for f1 in f1s))
        return [_cmul(val, twb_ref[z, f1, 0], twb_ref[z, f1, 1]) if f1 else val for val, f1 in zip(vals, f1s)]

    def outer(j, odd):
        rows = [FFT_PITCH * a + 16 * j for a in range(16)]
        cols = [_dft4(load(odd, 2, rows[n::4], 0, 16)) for n in range(4)]
        for k in range(4):
            store(odd, 2, rows[k::4], twiddle(dft16_row([col[k] for col in cols], k), j, range(k, 16, 4)), 0)

    def inner(half, e, odd, inverse):
        rows = [8 * FFT_PITCH * half + 2 * b for b in range(e, 128, 16)]
        cols = []
        for n in range(2):
            vals = load(odd, FFT_PITCH, rows[n::2], inverse, 0 if inverse else 16)
            cols.append(_dft4(rotate(vals, [e * g for g in range(n, 8, 2)], 16) if inverse else vals))
        for k in range(2):
            lo, hi = cols[1][k::2]
            if k:
                lo, hi = rotate([lo, hi], [16, 48], 16)
            (y0, y2), (y1, y3) = _butterfly(cols[0][k], lo), _butterfly(cols[0][k + 2], hi, k == 0)
            out = [y0, y1, y2, y3]
            out = out if inverse else rotate(out, [e * g for g in range(k, 8, 2)])
            store(odd, FFT_PITCH, rows[k::2], out, inverse)

    def centre(half, g1, odd):
        rows = [8 * FFT_PITCH * half + 2 * b for b in range(16 * g1, 16 * g1 + 16)]
        for n in range(4):
            park(0, n, _dft4(load(odd, FFT_PITCH, rows[n::4], 0, 16)))
        for k in range(4):
            vals = []
            for g2, val in zip(range(k, 16, 4), dft16_row(parked(0, k), k)):
                if g2 // 4 % 2 == 0:
                    z = 2 * half + odd + gate(w_ref.at[0, 0, 128], 12 if g2 < 4 else 28)
                vals.append(_cmul(val, w_ref[z, 0, g1 + 8 * g2], w_ref[z, 1, g1 + 8 * g2])[::-1])
            park(1, k, _dft4(vals))
        for k in range(4):
            store(odd, FFT_PITCH, rows[k::4], dft16_row(parked(1, k), k), 1)

    def outer_inverse(j, odd):
        rows = [FFT_PITCH * a + 16 * j for a in range(16)]
        for n in range(4):
            park(odd, n, _dft4(twiddle(load(odd, 2, rows[n::4], 1, 16), j, range(n, 16, 4))))
        for k in range(4):
            for a, (im, re) in zip(range(k, 16, 4), dft16_row(parked(odd, k), k)):
                im = pltpu.roll(im if odd else jnp.where(lane[:8] == 0, n_ref[j, a], im), 1 + odd, 1)
                g_ref[2 * odd, 8 * a:8 * a + 8, :] = jnp.where(own[odd][:8], re, im)
                g_ref[2 * odd + 1, 8 * a:8 * a + 8, :] = jnp.where(own[odd][:8], im, re)

    def nyquist():
        def factor(lo, n):
            return jnp.concatenate([nyq_ref[lo:lo + n, :], nyq_ref[lo + 48:lo + 48 + n, :]], axis=1)

        z = jnp.concatenate([n_ref[:, t].reshape(128, 128).T[0:1] for t in range(16)], axis=0)
        z = _dot(nyq_ref[0:256, 0:16], z)
        z = jnp.concatenate(_cmul((z[:128], z[128:]), tw_ref[0:128, :], tw_ref[128:256, :]), axis=1)
        yield
        w = [jnp.concatenate([wf_ref[i, 256:257, _tile(t)].astype(F32) for t in range(16)], axis=0) for i in range(2)]
        z = _dot_nt(factor(512, 32), z)
        z = jnp.concatenate(_cmul((z[:16], z[16:]), *w), axis=0)
        yield
        z = _dot(nyq_ref[256:512, 0:32], z)
        z = jnp.concatenate(_cmul((z[128:], z[:128]), tw_ref[0:128, :], tw_ref[128:256, :])[::-1], axis=1)
        yield
        z = _dot_nt(factor(544, 16), z)
        for t in range(16):
            n_ref[:, t] = jnp.broadcast_to(z[t:t + 1], (128, 128)).T.reshape(16, 8, 128)
        yield

    arrive()
    transpose_weights(0, 0, 2)
    slot = lax.broadcasted_iota(jnp.int32, (DH, 48), 1)
    probe = jnp.where(slot == 16, MAGIC, jnp.where(slot == 24, -MAGIC, jnp.where(slot >= 32, LOW, 0.0)))
    probe = jnp.where(slot < 16, jnp.where(slot % 5 == 1, 1.0 / 16 + GRID / 8, 1.0 / 16), probe)
    probe = _dot(probe.astype(BF16), jnp.ones((48, 512), BF16))
    peak_ref[...] = jnp.zeros(peak_ref.shape, F32)
    for j in range(4):
        peak_ref[3, 8 * j:8 * j + 8] = jnp.where(probe[0:8, _tile(j)] == 1.0 + 16 * LOW, 1.0, 0.0)

    arrive()
    for t in range(3):
        project(0, t, 0, 16)

    arrive()
    project(0, 3, 0, 16)
    transpose_weights(0, 2, 4)
    for t in range(4):
        project(0, t, 16, H)

    arrive()
    for f1 in range(1, 16):
        tw = jnp.broadcast_to(tw_ref[...][:, f1:f1 + 1], (256, 128)).reshape(2, 16, 8, 128)
        for p in range(2):
            twb_ref[:, f1, p] = tw[p]
    for t in range(4, 8):
        project(0, t)

    arrive()
    for t in range(8, 14):
        project(0, t)

    arrive()
    transpose_weights(1)
    finish(projections([(0, 14), (0, 15)] + [(1, t) for t in range(8)], spread(pairs(0, 2), 4, 8)))

    arrive()
    steps = spread([functools.partial(split_rows, r) for r in range(0, S, 16)], 0, 4.5)
    steps += [(64 * 5 - 1, functools.partial(forward, a)) for a in range(16)]
    finish(projections([(1, t) for t in range(8, 14)], steps))

    arrive()
    transpose_weights(2)
    column = nyquist()
    steps = spread(pairs(2, 8), 1, 15.5)
    steps += spread([functools.partial(filter_weights, i, t) for t in range(16) for i in range(2)], 1, 15.5)
    steps += [(64 * t - 1, lambda _: next(column)) for t in (5, 8, 10, 12)]
    stream = projections([(1, 14), (1, 15)] + [(2, t, 0, H if t < 12 else 24) for t in range(16)], steps)
    start(stream, 32 * 258, 64 * 16.6)
    for j in range(16):
        for odd in range(2):
            outer(j, odd)
    finish(stream)

    def save(h, block, o, den):
        for j in range(4):
            o_ref[4 * block + j, h] = o[:, _tile(j)]
            den_ref[4 * block + j, pl.ds(h, 8, stride=SUM_PITCH), :] = den[:, _tile(j)]

    def attention(half, it, between):
        v_words = v_refs[half].bitcast(U32)
        probs, done = [], 0
        for t in range(256):
            while done < min(4 * (t + 1) + LOOKAHEAD, 1024):
                unit, lo = divmod(done, 64)
                hi = min(4 * (t + 1) + LOOKAHEAD - 64 * unit, 64)
                hz = 4 * it + unit // 4 + zero()
                q = jnp.concatenate([q_words[16 * half + hz, 4 * (unit % 4) + j] for j in range(4)], axis=1)
                both = _dot(pltpu.bitcast(k_refs[half][hz, 8 * lo:8 * hi, 0:48], BF16),
                            pltpu.bitcast(jnp.concatenate([q, ones, q], axis=0), BF16))
                upper = (both + MAGIC) - MAGIC
                pair = jnp.exp2(upper), jnp.exp2((both - upper) * (1.0 / LOW))
                probs += [p[8 * r:8 * r + 8] for r in range(2 * (hi - lo)) for p in pair]
                done += hi - lo
            between(t)
            unit, keys = divmod(t, 16)
            h = 4 * it + unit // 4
            tile, probs = probs[:16], probs[16:]
            for i, p in enumerate(tile):
                den = p if keys == 0 and i == 0 else den + p
                if i == (5, 10)[half]:
                    yield lambda: den[:, _tile(3 - half)]
            o = _dot(pltpu.bitcast(v_words[h + zero(), keys], BF16), jnp.concatenate(tile[::-1], axis=0))
            acc = o + acc if keys else o
            if keys == 15:
                save(16 * half + h, unit % 4, acc, den)

    def guard():
        bound = jnp.max(peak_ref[0], axis=1, keepdims=True) * jnp.max(peak_ref[1], axis=1, keepdims=True)
        safe = (bound < (0.98 * RANGE / QSCALE) ** 2) & (peak_ref[2] < 2.0 ** 80)
        return jnp.min(jnp.where(safe, peak_ref[3], 0.0))

    def first_heads(it, carry):
        def between(t):
            if t % 7 == 6 and t < 7 * 32:
                pair_keys(1, 4 * it + t // 56, t // 7 % 8, pace["result"]())
            if t == 253:
                project(2, 12 + it, 24, H)

        stream = attention(0, it, between)
        start(stream, 8 * 32 + 32 * 95 + 8 * 432, 252, 2)
        for part in range(2):
            for t in range(4):
                z = gate(sq_ref.at[32, pl.ds(0, 8)], 32)
                peak_ref[part] = jnp.maximum(peak_ref[part], sublane_sum(sq_ref, 16 * part + 4 * it + t + z))
        half, odd = it // 2, it % 2
        for e in range(16):
            inner(half, e, odd, 0)
        for g1 in range(8):
            centre(half, g1, odd)
        for e in range(16):
            inner(half, e, odd, 1)
        finish(stream)
        return carry

    def last_heads(it, _):
        def between(t):
            if t % 64 == 61:
                backward(4 * it + t // 64)

        safe = guard()
        stream = attention(1, it, between)
        start(stream, 2 * 258, 54)
        for j in range(4):
            pace["clock"] = 64 * j + 2
            for odd in range(2):
                outer_inverse(4 * it + j, odd)
        finish(stream)
        filtered_rows(it).start()
        return safe

    def exact_attention(i, carry):
        h, block = i // 4, i % 4
        q = jnp.concatenate([q_ref[h, 4 * block + j] for j in range(4)], axis=1)
        k = pltpu.bitcast(jnp.where(h < 16, *(ref[h % 16, :, 0:48] for ref in k_refs)), BF16)
        pair = _dot(k[:, 0:DH], q), _dot(k[:, 32:48], q) * (1.0 / LOW)
        top = jnp.max(jnp.maximum(*pair), axis=0, keepdims=True)
        pair = [jnp.exp2(s - top) for s in pair]
        p = jnp.concatenate([x[64 * t + 8 * r:64 * t + 8 * r + 8] for t in range(16) for r in range(7, -1, -1)
                             for x in pair[::-1]], axis=0)
        v = [jnp.concatenate([ref[h % 16, t].astype(F32) for t in range(16)], axis=1) for ref in v_refs]
        save(h, block, _dot(jnp.where(h < 16, *v), p), jnp.sum(p.reshape(256, 8, 512), axis=0))
        return carry

    lax.fori_loop(0, 4, first_heads, 0)
    safe = lax.fori_loop(0, 4, last_heads, jnp.float32(0.0))

    @pl.when(safe < 0.5)
    def _():
        lax.fori_loop(0, 4 * H, exact_attention, 0)

    copies = [filtered_rows(i) for i in range(4)]
    edges = (0, 1, 4, 8, 12, 14, 15, 16)
    for lo, hi in zip(edges, edges[1:]):
        rows = []
        for t in range(lo, hi):
            inv_ref[t, :, 0:128] = 1.0 / sublane_sum(den_ref, t)
            o = [o_ref[t, h] * jnp.broadcast_to(inv_ref[t, h:h + 1, 0:128], (DH, 128)) for h in range(H)]
            rows.append(jnp.concatenate(o, axis=0).astype(BF16).T)
        o = jnp.concatenate(rows, axis=0)
        width = 128 if hi == 16 else D
        for c in range(0, D, width):
            tiles, cols = pl.ds(lo, hi - lo), pl.ds(c, width)
            ya_ref[tiles, :, cols] = _dot(o, wo_ref[:, cols]).astype(BF16).reshape(hi - lo, 128, width)
            copies.append(pltpu.make_async_copy(ya_ref.at[tiles, :, cols], out_hbm.at[tiles, :, cols], out_sem))
            copies[-1].start()
    for copy in copies:
        copy.wait()


@jax.jit
def pallas_concat_heads__mha_block__spectral_gfnet__prompt_kernel(
    A_x: jax.Array,
    A_wqkv: jax.Array,
    A_wo: jax.Array,
    B_x: jax.Array,
    B_w_r: jax.Array,
    B_w_i: jax.Array,
):
    vmem = pltpu.VMEM
    scratch = [
        vmem((S, D), BF16), vmem((3, D, D), BF16), vmem((D, D), BF16),
        vmem((1, S + 16, D), BF16), vmem((3, D // 2 + 1, S), BF16),
        vmem(_DFT.shape, BF16), vmem(_NYQUIST.shape, BF16), vmem(_TWIDDLES.shape, F32), vmem(_ROOTS.shape, F32),
        vmem((1, D // 2, D), U32), vmem((1, D // 2, D), U32), vmem((1, D // 2, D), U32),
        vmem((H, 16, DH, 128), BF16), vmem((H + 1, 16, DH, 128), BF16),
        vmem((16, 16, DH, 128), BF16), vmem((16, 16, DH, 128), BF16),
        vmem((16, S // 4, 128), U32), vmem((16, S // 4, 128), U32),
        vmem((33, 8 * SUM_PITCH + H, 128), F32), vmem((4, H, 128), F32),
        vmem((16, H, DH, 128), F32), vmem((16, 8 * SUM_PITCH + H, 128), F32),
        vmem((16, H, 256), F32),
        vmem((4, S, 128), BF16), vmem((2, 16 * FFT_PITCH + 256, 128), F32),
        vmem((3, 4, 4, 2, 8, 128), F32), vmem((4, 128, 128), F32),
        vmem((16, 16, 2, 8, 128), F32), vmem((4, 2, 132, 8, 128), F32), vmem((16, 16, 8, 128), F32),
        vmem((16, 128, D), BF16), vmem((16, 128, D), BF16),
        pltpu.SMEM((N_ZEROS,), jnp.int32), pltpu.SemaphoreType.DMA((9,)),
    ]
    out = pl.pallas_call(
        _kernel,
        out_shape=jax.ShapeDtypeStruct((16, 128, 2 * D), BF16),
        in_specs=[pl.BlockSpec(memory_space=pl.ANY)] * 10,
        out_specs=pl.BlockSpec(memory_space=pl.ANY),
        scratch_shapes=scratch,
        compiler_params=pltpu.CompilerParams(vmem_limit_bytes=100 * 1024 * 1024),
        name="mha_gfnet",
    )(A_x.reshape(S, D), A_wqkv, A_wo, B_x.reshape(S, D), B_w_r.T, B_w_i.T, _DFT, _NYQUIST, _TWIDDLES, _ROOTS)
    return out.reshape(1, S, 2 * D)
```

```python
import functools
import math

import jax
import jax.numpy as jnp
import numpy as np
from jax import lax
import jax.experimental.pallas as pl
import jax.experimental.pallas.tpu as pltpu

S, D, H, DH = 2048, 512, 32, 16
F32, BF16, U32 = jnp.float32, jnp.bfloat16, jnp.uint32

QSCALE = DH ** -0.5 * math.log2(math.e)
RANGE = 32.0
GRID = 2.0 ** -8
MAGIC = 1.5 * 2.0 ** 23 * GRID
LOW = GRID / (2.0 * RANGE)

FFT_PITCH = 260
SUM_PITCH = 36
N_ZEROS = 256
LOOKAHEAD = 8


def _constants():
    n = np.arange(128)[:, None]
    m = np.arange(64)[None, :]

    def cs(num, den):
        ang = 2.0 * np.pi * (num % den) / den
        return np.cos(ang), -np.sin(ang)

    def interleave(re, im, shift):
        return np.roll(np.stack([re, im], axis=2).reshape(128, 128), shift, axis=1)

    mats = [interleave(*cs(n * 4 * m, D), 0), interleave(*cs(n * (4 * m + 2), D), 1)]
    for first in (1, 5):
        mat = np.zeros((128, 128))
        for lane in range(128):
            k = 2 * lane + 1
            if first in (k % 8, -k % 8):
                c, s = cs(n[:64, 0] * (k if k % 8 == first else D - k), D)
                mat[:, lane] = np.concatenate([c, -s])
                mat[:, (lane + 2) % 128] = np.concatenate([s, c]) * (1.0 if k % 8 == first else -1.0)
        mats.append(mat)
    mats += [mat.T * (2.0 / (S * D)) for mat in mats]
    mats[0][:, 1] = (-1.0) ** np.arange(128)
    mats[4][0], mats[4][1] = 1.0 / (S * D), mats[0][:, 1] / (S * D)

    c, s = cs(n * np.arange(16)[None, :], 16)
    nyquist = np.zeros((640, 128))
    nyquist[:256, :16] = np.concatenate([c, s])
    nyquist[256:512, :32] = np.block([[c, s], [-s, c]])
    nyquist[512:608] = np.concatenate([c.T, s.T, c.T, -s.T, c.T, s.T])
    twiddles = np.concatenate(cs(n * n.T, S))
    roots = np.zeros((1, 144, 256))
    roots[0, :128, :128], roots[0, :128, 128:] = cs(n, 128)
    return (np.stack(mats).astype(jnp.bfloat16), nyquist.astype(jnp.bfloat16),
            twiddles.astype(np.float32), roots.astype(np.float32))


_DFT, _NYQUIST, _TWIDDLES, _ROOTS = _constants()


def _cmul(z, c, s):
    re, im = z
    return re * c - im * s, re * s + im * c


def _butterfly(a, b, quarter=False):
    (ar, ai), (br, bi) = a, b
    if quarter:
        return (ar + bi, ai - br), (ar - bi, ai + br)
    return (ar + br, ai + bi), (ar - br, ai - bi)


def _dft4(x, quarter=False):
    s0, d0 = _butterfly(x[0], x[2], quarter)
    s1, d1 = _butterfly(x[1], x[3])
    (y0, y2), (y1, y3) = _butterfly(s0, s1), _butterfly(d0, d1, True)
    return [y0, y1, y2, y3]


def _dot(a, b):
    return lax.dot_general(a, b, (((1,), (0,)), ((), ())), preferred_element_type=F32)


def _dot_nt(a, b):
    return lax.dot_general(a, b, (((1,), (1,)), ((), ())), preferred_element_type=F32)


def _unpack(both):
    upper = (both + MAGIC) - MAGIC
    return upper, (both - upper) * (1.0 / LOW)


def _tile(j):
    return slice(j * 128, (j + 1) * 128)


def _block(i, size):
    return pl.ds(i * size if isinstance(i, int) else pl.multiple_of(i * size, size), size)


def _kernel(ax_hbm, wqkv_hbm, wo_hbm, bx_hbm, wr_hbm, wi_hbm, dft_hbm, nyq_hbm, tw_hbm, roots_hbm, out_hbm,
            ax_ref, wqkv_ref, wo_ref, bx_ref, wf_ref, dft_ref, nyq_ref, tw_ref, roots_ref,
            wq_ref, wk_ref, wv_ref, q_ref, kt_ref, v0_ref, v1_ref, k0_ref, k1_ref, sq_ref, peak_ref,
            o_ref, den_ref, inv_ref, u_ref, f_ref, t_ref, g_ref, twb_ref, w_ref, n_ref, ya_ref, yb_ref, zero_ref, sems):
    def x_tiles(lo, hi):
        rows = pl.ds(128 * lo, 128 * (hi - lo))
        return ax_hbm.at[rows], ax_ref.at[rows]

    def w_part(i, lo=0, n=D):
        return wqkv_hbm.at[:, pl.ds(i * D + lo, n)], wqkv_ref.at[i, :, pl.ds(lo, n)]

    stages = [[w_part(0, 0, 256)], [x_tiles(0, 3)], [x_tiles(3, 4), w_part(0, 256, 256)],
              [x_tiles(4, 8), (tw_hbm, tw_ref)], [x_tiles(8, 14)], [x_tiles(14, 16), w_part(1)],
              [(dft_hbm, dft_ref), (bx_hbm, bx_ref.at[0, pl.ds(0, S)])],
              [w_part(2), (roots_hbm, roots_ref), (wr_hbm, wf_ref.at[0]), (wi_hbm, wf_ref.at[1]),
               (nyq_hbm, nyq_ref), (wo_hbm, wo_ref)]]
    stages = [[pltpu.make_async_copy(src, dst, sems.at[i]) for src, dst in stage] for i, stage in enumerate(stages)]
    out_sem = sems.at[len(stages)]
    for stage in stages:
        for copy in stage:
            copy.start()

    def arrive():
        for copy in stages.pop(0):
            copy.wait()

    def fill(i, carry):
        for j in range(8):
            zero_ref[i * 8 + j] = 0
        return carry

    lax.fori_loop(0, N_ZEROS // 8, fill, 0)
    pace = {"zeros": 0}

    def zero():
        pace["zeros"] += 1
        return zero_ref[pace["zeros"] % N_ZEROS]

    def start(stream, ops, ticks, first=0.0):
        pace.update(stream=stream, clock=first, rate=ops / ticks, tick=-1)

    def gate(spare, ops):
        while pace["tick"] < int(pace["clock"]):
            pace["result"] = next(pace["stream"])
            pace["tick"] += 1
        spare[...] = pace["result"]()
        pace["clock"] += ops / pace["rate"]
        return zero()

    def finish(stream):
        for _ in stream:
            pass

    w_refs, k_refs, v_refs = (wq_ref, wk_ref, wv_ref), (k0_ref, k1_ref), (v0_ref, v1_ref)
    q_words, kt_words = q_ref.bitcast(U32), kt_ref.bitcast(U32)

    def transpose_weights(part, lo=0, hi=4):
        for j in range(lo, hi):
            w_refs[part][0, 64 * j:64 * j + 64, :] = pltpu.bitcast(wqkv_ref[part, :, _tile(j)].T, U32)

    def project(part, t, lo=0, hi=H):
        if part == 1:
            groups = [32 * (t // 2) + 16 * (r // 8) + 15 - 2 * (r % 8) - t % 2 for r in range(16)]
            x = jnp.concatenate([ax_ref[8 * g:8 * g + 8, :].astype(F32) for g in groups], axis=0).astype(BF16)
        else:
            x = ax_ref[_block(t, 128), :]
        y = _dot_nt(pltpu.bitcast(w_refs[part][zero(), 8 * lo:8 * hi, :], BF16), x)
        z = y.reshape(hi - lo, DH, 128)
        if part == 2:
            if lo == 0:
                v0_ref[:, t] = z[:16].astype(BF16)
            v1_ref[max(lo - 16, 0):hi - 16, t] = z[max(16 - lo, 0):].astype(BF16)
            peak_ref[2, 0:8] = jnp.maximum(peak_ref[2, 0:8], jnp.max(jnp.abs(y).reshape(-1, 8, 128), axis=0))
            return y
        if part == 0:
            q_ref[lo:hi, t] = (z * QSCALE).astype(BF16)
        else:
            kt_ref[0:H, t] = (z * LOW if t % 2 else z).astype(BF16)
        square = z * z
        square = square[:, :8] + square[:, 8:]
        for h in range(lo, hi):
            sq_ref[16 * part + t, pl.ds(h, 8, stride=SUM_PITCH), :] = square[h - lo]
        return y

    def projections(jobs, steps):
        steps, tick = sorted(steps, key=lambda step: step[0]), -1
        for job in jobs:
            y = project(*job)
            for r in range(0, y.shape[0], 8):
                tick += 1
                while steps and steps[0][0] <= tick:
                    steps.pop(0)[1](y[r:r + 8])
                yield lambda: y[r:r + 8]
        assert not steps

    def spread(steps, lo, hi):
        return [(64 * (lo + (hi - lo) * i / len(steps)), step) for i, step in enumerate(steps)]

    def sublane_sum(ref, t):
        return functools.reduce(jnp.add, [ref[t, SUM_PITCH * r:SUM_PITCH * r + H, :] for r in range(8)])

    row = lax.broadcasted_iota(jnp.int32, (DH, 128), 0)
    magic = pltpu.bitcast(jnp.where(row == 0, MAGIC, jnp.where(row == 8, -MAGIC, 0.0)).astype(BF16), U32)
    ones = pltpu.bitcast(jnp.ones((DH, 512), BF16), U32)

    def pair_keys(half, h, t, after):
        kt_words[H, 0] = pltpu.bitcast(after, U32)
        hz = 16 * half + h + zero()
        both = jnp.concatenate([kt_words[hz, 2 * t], magic, kt_words[hz, 2 * t + 1]], axis=0)
        k_refs[half][h, 64 * t:64 * t + 64, 0:48] = pltpu.bitcast(pltpu.bitcast(both, BF16).T, U32)

    def pairs(lo, hi):
        return [functools.partial(pair_keys, 0, h, t) for t in range(lo, hi) for h in range(16)]

    lane = lax.broadcasted_iota(jnp.int32, (128, 128), 1)
    left = lane < 64
    own = (lane % 2 == 0, (lane + 1) % 4 < 2)
    dft_words, u_words = dft_ref.bitcast(U32), u_ref.bitcast(U32)

    def dft_matrix(i):
        return pltpu.bitcast(dft_words[i], BF16)

    def split_rows(r, after):
        bx_ref[0, S:S + 8, 0:128] = after.astype(BF16)
        x = bx_ref[zero(), r:r + 16, :].astype(F32)
        x0, x1, x2, x3 = (x[:, _tile(i)] for i in range(4))
        e0, e1, o0, o1 = x0 + x2, x1 + x3, x0 - x2, x3 - x1
        p = jnp.where(left[:16], o0, pltpu.roll(o1, 64, 1))
        q = jnp.where(left[:16], pltpu.roll(o0 + o1, 64, 1), o1 - o0) * math.sqrt(0.5)
        for i, val in enumerate((e0 + e1, e0 - e1, p + q, p - q)):
            u_ref[i, r:r + 16, :] = val.astype(BF16)

    def forward(a, _):
        z = zero()
        y = [_dot(pltpu.bitcast(u_words[i, 64 * a:64 * a + 64, :], BF16), dft_matrix(z + i)) for i in range(4)]
        for odd in range(2):
            im = pltpu.roll(jnp.where(own[odd], y[2 * odd + 1], y[2 * odd]), 127 - odd, 1)
            if not odd:
                n_ref[:, a] = im.reshape(16, 8, 128)
                im = jnp.where(lane == 0, 0.0, im)
            f_ref[odd, pl.ds(FFT_PITCH * a, 128, stride=2), :] = jnp.where(own[odd], y[2 * odd], y[2 * odd + 1])
            f_ref[odd, pl.ds(FFT_PITCH * a + 1, 128, stride=2), :] = im

    def backward(j):
        z = zero()
        y = [_dot(g_ref[z + i], dft_matrix(z + 4 + i)) for i in range(4)]
        e0, e1, p, q = y[0] + y[1], y[0] - y[1], y[2] + y[3], (y[2] - y[3]) * math.sqrt(0.5)
        turned = pltpu.roll(q, 64, 1)
        o0, o1 = jnp.where(left, p, turned - q), jnp.where(left, pltpu.roll(p, 64, 1), turned + q)
        y = jnp.concatenate([e0 + o0, e1 - o1, e0 - o0, e1 + o1], axis=1).astype(BF16)
        yb_ref[:, _block(j, 8), :] = y.reshape(16, 8, D)

    def filtered_rows(i):
        rows = _block(i, 32)
        return pltpu.make_async_copy(yb_ref.at[:, rows], out_hbm.at[:, rows, pl.ds(D, D)], out_sem)

    def filter_weights(i, t, after):
        wf_ref[2, 0:8, 0:128] = after.astype(BF16)
        w = pltpu.bitcast(wf_ref[i + zero(), 0:256, _tile(t)], U32).T.reshape(8, 2, 8, 128)
        for half in range(2):
            w_ref[2 * half, i, 8 * t:8 * t + 8] = pltpu.bitcast(w[:, half] << 16, F32)
            w_ref[2 * half + 1, i, 8 * t:8 * t + 8] = pltpu.bitcast(w[:, half] & np.uint32(0xFFFF0000), F32)

    def load(odd, stride, rows, swap, ops):
        z = odd + gate(f_ref.at[0, pl.ds(16 * FFT_PITCH, 8)], ops)
        return [tuple(f_ref[z, pl.ds(r + (p ^ swap), 8, stride=stride), :] for p in range(2)) for r in rows]

    def store(odd, stride, rows, vals, swap):
        z = odd + zero()
        for r, val in zip(rows, vals):
            for p in range(2):
                f_ref[z, pl.ds(r + (p ^ swap), 8, stride=stride), :] = val[p]

    def park(slot, n, vals):
        for k, val in enumerate(vals):
            for p in range(2):
                t_ref[slot, k, n, p] = val[p]

    def parked(slot, k):
        z = slot + gate(t_ref.at[2, 0, 0, 0], 0)
        return [(t_ref[z, k, n, 0], t_ref[z, k, n, 1]) for n in range(4)]

    def rotate(vals, ks, ops=0):
        z = gate(roots_ref.at[0, pl.ds(128, 8), pl.ds(0, 128)],
                 ops + sum(0 if k == 0 else 4 if k % 32 == 16 else 6 for k in ks))
        out = []
        for (re, im), k in zip(vals, ks):
            if k == 0:
                out.append((re, im))
                continue
            c = jnp.broadcast_to(roots_ref[z, k:k + 1, _tile(0)], (8, 128))
            if k % 64 == 16:
                out.append(((re + im) * c, (im - re) * c))
            elif k % 64 == 48:
                out.append(((re - im) * c, (re + im) * c))
            else:
                out.append(_cmul((re, im), c, jnp.broadcast_to(roots_ref[z, k:k + 1, _tile(1)], (8, 128))))
        return out

    def dft16_row(vals, k):
        return _dft4(rotate(vals, [0 if n * k == 4 else 8 * n * k for n in range(4)], 16), k == 2)

    def twiddle(vals, j, f1s):
        z = j + gate(twb_ref.at[0, 0, 0], 6 * sum(f1 > 0 for f1 in f1s))
        return [_cmul(val, twb_ref[z, f1, 0], twb_ref[z, f1, 1]) if f1 else val for val, f1 in zip(vals, f1s)]

    def outer(j, odd):
        rows = [FFT_PITCH * a + 16 * j for a in range(16)]
        cols = [_dft4(load(odd, 2, rows[n::4], 0, 16)) for n in range(4)]
        for k in range(4):
            store(odd, 2, rows[k::4], twiddle(dft16_row([col[k] for col in cols], k), j, range(k, 16, 4)), 0)

    def inner(half, e, odd, inverse):
        rows = [8 * FFT_PITCH * half + 2 * b for b in range(e, 128, 16)]
        cols = []
        for n in range(2):
            vals = load(odd, FFT_PITCH, rows[n::2], inverse, 0 if inverse else 16)
            cols.append(_dft4(rotate(vals, [e * g for g in range(n, 8, 2)], 16) if inverse else vals))
        for k in range(2):
            lo, hi = cols[1][k::2]
            if k:
                lo, hi = rotate([lo, hi], [16, 48], 16)
            (y0, y2), (y1, y3) = _butterfly(cols[0][k], lo), _butterfly(cols[0][k + 2], hi, k == 0)
            out = [y0, y1, y2, y3]
            out = out if inverse else rotate(out, [e * g for g in range(k, 8, 2)])
            store(odd, FFT_PITCH, rows[k::2], out, inverse)

    def centre(half, g1, odd):
        rows = [8 * FFT_PITCH * half + 2 * b for b in range(16 * g1, 16 * g1 + 16)]
        for n in range(4):
            park(0, n, _dft4(load(odd, FFT_PITCH, rows[n::4], 0, 16)))
        for k in range(4):
            vals = []
            for g2, val in zip(range(k, 16, 4), dft16_row(parked(0, k), k)):
                if g2 // 4 % 2 == 0:
                    z = 2 * half + odd + gate(w_ref.at[0, 0, 128], 12 if g2 < 4 else 28)
                vals.append(_cmul(val, w_ref[z, 0, g1 + 8 * g2], w_ref[z, 1, g1 + 8 * g2])[::-1])
            park(1, k, _dft4(vals))
        for k in range(4):
            store(odd, FFT_PITCH, rows[k::4], dft16_row(parked(1, k), k), 1)

    def outer_inverse(j, odd):
        rows = [FFT_PITCH * a + 16 * j for a in range(16)]
        for n in range(4):
            park(odd, n, _dft4(twiddle(load(odd, 2, rows[n::4], 1, 16), j, range(n, 16, 4))))
        for k in range(4):
            for a, (im, re) in zip(range(k, 16, 4), dft16_row(parked(odd, k), k)):
                im = pltpu.roll(im if odd else jnp.where(lane[:8] == 0, n_ref[j, a], im), 1 + odd, 1)
                g_ref[2 * odd, 8 * a:8 * a + 8, :] = jnp.where(own[odd][:8], re, im)
                g_ref[2 * odd + 1, 8 * a:8 * a + 8, :] = jnp.where(own[odd][:8], im, re)

    def nyquist():
        def factor(lo, n):
            return jnp.concatenate([nyq_ref[lo:lo + n, :], nyq_ref[lo + 48:lo + 48 + n, :]], axis=1)

        z = jnp.concatenate([n_ref[:, t].reshape(128, 128).T[0:1] for t in range(16)], axis=0)
        z = _dot(nyq_ref[0:256, 0:16], z)
        z = jnp.concatenate(_cmul((z[:128], z[128:]), tw_ref[0:128, :], tw_ref[128:256, :]), axis=1)
        yield
        w = [jnp.concatenate([wf_ref[i, 256:257, _tile(t)].astype(F32) for t in range(16)], axis=0) for i in range(2)]
        z = _dot_nt(factor(512, 32), z)
        z = jnp.concatenate(_cmul((z[:16], z[16:]), *w), axis=0)
        yield
        z = _dot(nyq_ref[256:512, 0:32], z)
        z = jnp.concatenate(_cmul((z[128:], z[:128]), tw_ref[0:128, :], tw_ref[128:256, :])[::-1], axis=1)
        yield
        z = _dot_nt(factor(544, 16), z)
        for t in range(16):
            n_ref[:, t] = jnp.broadcast_to(z[t:t + 1], (128, 128)).T.reshape(16, 8, 128)
        yield

    arrive()
    transpose_weights(0, 0, 2)
    slot = lax.broadcasted_iota(jnp.int32, (DH, 48), 1)
    probe = jnp.where(slot == 16, MAGIC, jnp.where(slot == 24, -MAGIC, jnp.where(slot >= 32, LOW, 0.0)))
    probe = jnp.where(slot < 16, jnp.where(slot % 5 == 1, 1.0 / 16 + GRID / 8, 1.0 / 16), probe)
    upper, lower = _unpack(_dot(probe.astype(BF16), jnp.ones((48, 512), BF16)))
    probe = jnp.where((upper == 1.0) & (lower == 16.0), 1.0, 0.0)
    peak_ref[...] = jnp.zeros(peak_ref.shape, F32)
    for j in range(4):
        peak_ref[3, 8 * j:8 * j + 8] = probe[0:8, _tile(j)]

    arrive()
    for t in range(3):
        project(0, t, 0, 16)

    arrive()
    project(0, 3, 0, 16)
    transpose_weights(0, 2, 4)
    for t in range(4):
        project(0, t, 16, H)

    arrive()
    for f1 in range(1, 16):
        tw = jnp.broadcast_to(tw_ref[...][:, f1:f1 + 1], (256, 128)).reshape(2, 16, 8, 128)
        for p in range(2):
            twb_ref[:, f1, p] = tw[p]
    for t in range(4, 8):
        project(0, t)

    arrive()
    for t in range(8, 14):
        project(0, t)

    arrive()
    transpose_weights(1)
    finish(projections([(0, 14), (0, 15)] + [(1, t) for t in range(8)], spread(pairs(0, 2), 4, 8)))

    arrive()
    steps = spread([functools.partial(split_rows, r) for r in range(0, S, 16)], 0, 4.5)
    steps += [(64 * 5 - 1, functools.partial(forward, a)) for a in range(16)]
    finish(projections([(1, t) for t in range(8, 14)], steps))

    arrive()
    transpose_weights(2)
    column = nyquist()
    steps = spread(pairs(2, 8), 1, 15.5)
    steps += spread([functools.partial(filter_weights, i, t) for t in range(16) for i in range(2)], 1, 15.5)
    steps += [(64 * t - 1, lambda _: next(column)) for t in (5, 8, 10, 12)]
    stream = projections([(1, 14), (1, 15)] + [(2, t, 0, H if t < 12 else 24) for t in range(16)], steps)
    start(stream, 32 * 258, 64 * 16.6)
    for j in range(16):
        for odd in range(2):
            outer(j, odd)
    finish(stream)

    def save(h, block, o, den):
        for j in range(4):
            o_ref[4 * block + j, h] = o[:, _tile(j)]
            den_ref[4 * block + j, pl.ds(h, 8, stride=SUM_PITCH), :] = den[:, _tile(j)]

    def attention(half, it, between):
        v_words = v_refs[half].bitcast(U32)
        probs, done = [], 0
        for t in range(256):
            while done < min(4 * (t + 1) + LOOKAHEAD, 1024):
                unit, lo = divmod(done, 64)
                hi = min(4 * (t + 1) + LOOKAHEAD - 64 * unit, 64)
                hz = 4 * it + unit // 4 + zero()
                q = jnp.concatenate([q_words[16 * half + hz, 4 * (unit % 4) + j] for j in range(4)], axis=1)
                both = _dot(pltpu.bitcast(k_refs[half][hz, 8 * lo:8 * hi, 0:48], BF16),
                            pltpu.bitcast(jnp.concatenate([q, ones, q], axis=0), BF16))
                pair = [jnp.exp2(s) for s in _unpack(both)]
                probs += [p[8 * r:8 * r + 8] for r in range(2 * (hi - lo)) for p in pair]
                done += hi - lo
            between(t)
            unit, keys = divmod(t, 16)
            h = 4 * it + unit // 4
            tile, probs = probs[:16], probs[16:]
            for i, p in enumerate(tile):
                den = p if keys == 0 and i == 0 else den + p
                if i == (5, 10)[half]:
                    yield lambda: den[:, _tile(3 - half)]
            o = _dot(pltpu.bitcast(v_words[h + zero(), keys], BF16), jnp.concatenate(tile[::-1], axis=0))
            acc = o + acc if keys else o
            if keys == 15:
                save(16 * half + h, unit % 4, acc, den)

    def guard():
        bound = jnp.max(peak_ref[0], axis=1, keepdims=True) * jnp.max(peak_ref[1], axis=1, keepdims=True)
        v = peak_ref[2]
        safe = (bound < (0.98 * RANGE / QSCALE) ** 2) & (v < 2.0 ** 80) & ((v > 2.0 ** -60) | (v == 0.0))
        return jnp.min(jnp.where(safe, peak_ref[3], 0.0))

    def first_heads(it, carry):
        def between(t):
            if t % 7 == 6 and t < 7 * 32:
                pair_keys(1, 4 * it + t // 56, t // 7 % 8, pace["result"]())
            if t == 253:
                project(2, 12 + it, 24, H)

        stream = attention(0, it, between)
        start(stream, 8 * 32 + 32 * 95 + 8 * 432, 252, 2)
        for part in range(2):
            for t in range(4):
                z = gate(sq_ref.at[32, pl.ds(0, 8)], 32)
                peak_ref[part] = jnp.maximum(peak_ref[part], sublane_sum(sq_ref, 16 * part + 4 * it + t + z))
        half, odd = it // 2, it % 2
        for e in range(16):
            inner(half, e, odd, 0)
        for g1 in range(8):
            centre(half, g1, odd)
        for e in range(16):
            inner(half, e, odd, 1)
        finish(stream)
        return carry

    def last_heads(it, _):
        def between(t):
            if t % 64 == 61:
                backward(4 * it + t // 64)

        safe = guard()
        stream = attention(1, it, between)
        start(stream, 2 * 258, 54)
        for j in range(4):
            pace["clock"] = 64 * j + 2
            for odd in range(2):
                outer_inverse(4 * it + j, odd)
        finish(stream)
        filtered_rows(it).start()
        return safe

    def exact_attention(i, carry):
        h, block = i // 4, i % 4
        q = jnp.concatenate([q_ref[h, 4 * block + j] for j in range(4)], axis=1)
        k = pltpu.bitcast(jnp.where(h < 16, *(ref[h % 16, :, 0:48] for ref in k_refs)), BF16)
        pair = _dot(k[:, 0:DH], q), _dot(k[:, 32:48], q) * (1.0 / LOW)
        top = jnp.max(jnp.maximum(*pair), axis=0, keepdims=True)
        pair = [jnp.exp2(s - top) for s in pair]
        p = jnp.concatenate([x[64 * t + 8 * r:64 * t + 8 * r + 8] for t in range(16) for r in range(7, -1, -1)
                             for x in pair[::-1]], axis=0)
        v = [jnp.concatenate([ref[h % 16, t].astype(F32) for t in range(16)], axis=1) for ref in v_refs]
        save(h, block, _dot(jnp.where(h < 16, *v), p), jnp.sum(p.reshape(256, 8, 512), axis=0))
        return carry

    lax.fori_loop(0, 4, first_heads, 0)
    safe = lax.fori_loop(0, 4, last_heads, jnp.float32(0.0))

    @pl.when(safe < 0.5)
    def _():
        lax.fori_loop(0, 4 * H, exact_attention, 0)

    copies = [filtered_rows(i) for i in range(4)]
    edges = (0, 1, 4, 8, 12, 14, 15, 16)
    for lo, hi in zip(edges, edges[1:]):
        rows = []
        for t in range(lo, hi):
            inv_ref[t, :, 0:128] = 1.0 / sublane_sum(den_ref, t)
            o = [o_ref[t, h] * jnp.broadcast_to(inv_ref[t, h:h + 1, 0:128], (DH, 128)) for h in range(H)]
            rows.append(jnp.concatenate(o, axis=0).astype(BF16).T)
        o = jnp.concatenate(rows, axis=0)
        width = 128 if hi == 16 else D
        for c in range(0, D, width):
            tiles, cols = pl.ds(lo, hi - lo), pl.ds(c, width)
            ya_ref[tiles, :, cols] = _dot(o, wo_ref[:, cols]).astype(BF16).reshape(hi - lo, 128, width)
            copies.append(pltpu.make_async_copy(ya_ref.at[tiles, :, cols], out_hbm.at[tiles, :, cols], out_sem))
            copies[-1].start()
    for copy in copies:
        copy.wait()


@jax.jit
def pallas_concat_heads__mha_block__spectral_gfnet__prompt_kernel(
    A_x: jax.Array,
    A_wqkv: jax.Array,
    A_wo: jax.Array,
    B_x: jax.Array,
    B_w_r: jax.Array,
    B_w_i: jax.Array,
):
    vmem = pltpu.VMEM
    scratch = [
        vmem((S, D), BF16), vmem((3, D, D), BF16), vmem((D, D), BF16),
        vmem((1, S + 16, D), BF16), vmem((3, D // 2 + 1, S), BF16),
        vmem(_DFT.shape, BF16), vmem(_NYQUIST.shape, BF16), vmem(_TWIDDLES.shape, F32), vmem(_ROOTS.shape, F32),
        vmem((1, D // 2, D), U32), vmem((1, D // 2, D), U32), vmem((1, D // 2, D), U32),
        vmem((H, 16, DH, 128), BF16), vmem((H + 1, 16, DH, 128), BF16),
        vmem((16, 16, DH, 128), BF16), vmem((16, 16, DH, 128), BF16),
        vmem((16, S // 4, 128), U32), vmem((16, S // 4, 128), U32),
        vmem((33, 8 * SUM_PITCH + H, 128), F32), vmem((4, H, 128), F32),
        vmem((16, H, DH, 128), F32), vmem((16, 8 * SUM_PITCH + H, 128), F32),
        vmem((16, H, 256), F32),
        vmem((4, S, 128), BF16), vmem((2, 16 * FFT_PITCH + 256, 128), F32),
        vmem((3, 4, 4, 2, 8, 128), F32), vmem((4, 128, 128), F32),
        vmem((16, 16, 2, 8, 128), F32), vmem((4, 2, 132, 8, 128), F32), vmem((16, 16, 8, 128), F32),
        vmem((16, 128, D), BF16), vmem((16, 128, D), BF16),
        pltpu.SMEM((N_ZEROS,), jnp.int32), pltpu.SemaphoreType.DMA((9,)),
    ]
    out = pl.pallas_call(
        _kernel,
        out_shape=jax.ShapeDtypeStruct((16, 128, 2 * D), BF16),
        in_specs=[pl.BlockSpec(memory_space=pl.ANY)] * 10,
        out_specs=pl.BlockSpec(memory_space=pl.ANY),
        scratch_shapes=scratch,
        compiler_params=pltpu.CompilerParams(vmem_limit_bytes=100 * 1024 * 1024),
        name="mha_gfnet",
    )(A_x.reshape(S, D), A_wqkv, A_wo, B_x.reshape(S, D), B_w_r.T, B_w_i.T, _DFT, _NYQUIST, _TWIDDLES, _ROOTS)
    return out.reshape(1, S, 2 * D)
```
